```python
import jax
import jax.numpy as jnp

def _softmax(x, axis=-1):
    return jax.nn.softmax(x, axis=axis)
def _gelu(x):
    return jax.nn.gelu(x, approximate=True)
def _silu(x):
    return jax.nn.silu(x)
def _sigmoid(x):
    return jax.nn.sigmoid(x)
def _layernorm(x, axis=-1, eps=1e-5):
    m = jnp.mean(x, axis=axis, keepdims=True)
    v = jnp.var(x, axis=axis, keepdims=True)
    return (x - m) / jnp.sqrt(v + eps)
def _scatter_add(tgt, idx, src, axis=0):
    return tgt.at[idx].add(src)
def _segment_sum(src, seg, n):
    return jax.ops.segment_sum(src, seg, n)
class _Rng:
    def __init__(self, key):
        self._k = key
    def _next(self):
        self._k, sub = jax.random.split(self._k)
        return sub
    def normal(self, shape):
        return jax.random.normal(self._next(), shape, dtype=jnp.bfloat16)
    def randint(self, lo, hi, shape):
        return jax.random.randint(self._next(), shape, lo, hi, dtype=jnp.int32)
    def uniform(self, shape, lo=0.0, hi=1.0):
        return jax.random.uniform(self._next(), shape, jnp.bfloat16, lo, hi)
    def permutation(self, n):
        return jax.random.permutation(self._next(), n)


kernel_name = 'parallel_sum__sliding_local_dilated__mixer_channel_mlp__prompt'

def _fwd_setup_inputs():
    _rng = _Rng(jax.random.key(int.from_bytes(__import__("os").urandom(4), "little")))
    _w = (lambda a: (lambda t: t.astype(jnp.bfloat16) if jnp.issubdtype(t.dtype, jnp.floating) else t)(jnp.asarray(a)))
    def _A_setup():
        B, S, D = 1, 2048, 576
        return {
            "x": _w((lambda *s: _rng.normal(s) * 0.05)(B, S, D)),
            "wqkv": _w((lambda *s: _rng.normal(s) * 0.05)(D, 3 * D)),
            "wo": _w((lambda *s: _rng.normal(s) * 0.05)(D, D)),
        }
    _A_in = _A_setup()

    def _B_setup():
        B, S, D, F = 1, 2048, 576, 4608
        return {
            "x": _w((lambda *s: _rng.normal(s) * 0.05)(B, S, D)),
            "w1": _w((lambda *s: _rng.normal(s) * 0.05)(D, F) * (D ** -0.5)),
            "b1": _w((lambda *s: _rng.normal(s) * 0.05)(F)),
            "w2": _w((lambda *s: _rng.normal(s) * 0.05)(F, D) * (F ** -0.5)),
            "b2": _w((lambda *s: _rng.normal(s) * 0.05)(D)),
        }
    _B_in = _B_setup()

    return {
        "A_x": _A_in["x"],
        "A_wqkv": _A_in["wqkv"],
        "A_wo": _A_in["wo"],
        "B_x": _B_in["x"],
        "B_w1": _B_in["w1"],
        "B_b1": _B_in["b1"],
        "B_w2": _B_in["w2"],
        "B_b2": _B_in["b2"],
    }

def _fwd_reference(A_x, A_wqkv, A_wo, B_x, B_w1, B_b1, B_w2, B_b2):
    def _A_ref(x, wqkv, wo):
        B, S, D = x.shape
        H = 32; Dh = D // H
        W, dil = 8, 2
        qkv = (lambda x, *d: x.transpose(*d))((x @ wqkv).reshape(B, S, 3, H, Dh), 2, 0, 3, 1, 4)
        q, k, v = qkv[0], qkv[1], qkv[2]
        scale = Dh ** -0.5
        pos = jnp.arange(S)
        off = jnp.arange(W) * dil
        idx = pos[:, None] - off[None, :]
        mask = idx >= 0
        idx_c = jnp.where(mask, idx, 0).reshape(-1)
        kg = k[:, :, idx_c, :].reshape(B, H, S, W, Dh)
        vg = v[:, :, idx_c, :].reshape(B, H, S, W, Dh)
        logits = jnp.einsum("bhsd,bhswd->bhsw", q, kg) * scale
        logits = jnp.where(mask[None, None, :, :], logits, -1e9)
        attn = _softmax(logits, axis=-1)
        o = jnp.einsum("bhsw,bhswd->bhsd", attn, vg)
        return (lambda x, *d: x.transpose(*d))(o, 0, 2, 1, 3).reshape(B, S, D) @ wo

    def _B_ref(x, w1, b1, w2, b2):
        y = _layernorm(x, axis=-1)
        h = _gelu(jnp.einsum("bsd,df->bsf", y, w1) + b1)
        return jnp.einsum("bsf,fd->bsd", h, w2) + b2

    x = A_x
    xn = _layernorm(x, axis=-1)
    return x + _A_ref(xn, A_wqkv, A_wo) + _B_ref(xn, B_w1, B_b1, B_w2, B_b2)


def setup_inputs():
    _inp = _fwd_setup_inputs()
    _gk = jax.random.fold_in(jax.random.key(int.from_bytes(__import__("os").urandom(4), "little")), 2**31 - 1)
    _shapes = [[1, 2048, 576]]
    _dtypes = ['bfloat16']
    _gks = jax.random.split(_gk, len(_shapes))
    _gs = [jax.random.normal(k, s, dtype=jnp.dtype(d)) * 0.05 for k, s, d in zip(_gks, _shapes, _dtypes)]
    _inp["grad_out"] = _gs[0]
    return _inp

def reference(A_x, A_wqkv, A_wo, B_w1, B_b1, B_w2, B_b2, B_x, grad_out):
    _const = dict(B_x=B_x)
    def _f(*_d):
        return _fwd_reference(**{'A_x': _d[0], 'A_wqkv': _d[1], 'A_wo': _d[2], 'B_w1': _d[3], 'B_b1': _d[4], 'B_w2': _d[5], 'B_b2': _d[6], **_const})
    _out, _vjp = jax.vjp(_f, A_x, A_wqkv, A_wo, B_w1, B_b1, B_w2, B_b2)
    _grads = _vjp(grad_out)
    _out0 = jnp.asarray(_out)
    return (_out0, *[jnp.asarray(_g) for _g in _grads])
```

```python
import functools
import jax
import jax.numpy as jnp
import jax.experimental.pallas as pl
import jax.experimental.pallas.tpu as pltpu

S, D, F = 2048, 576, 4608
H, DH, W, DIL = 32, 18, 8, 2
DP = 640
NQ = 14
QP = NQ * 128
PAD = 16
EPS = 1e-5
SCALE = DH ** -0.5
C0 = 0.7978845608028654
C1 = 0.044715
NEG = -1e9

TF = 256
NF = F // TF
TB = 256
NB = S // TB
RA = 16
RS = 128
NSL = S // RS

f32 = jnp.float32
bf16 = jnp.bfloat16


def NN(a, b):
    return jax.lax.dot_general(a, b, (((1,), (0,)), ((), ())), preferred_element_type=f32)


def NT(a, b):
    return jax.lax.dot_general(a, b, (((1,), (1,)), ((), ())), preferred_element_type=f32)


GROUPS = ([(0, d) for d in range(16)] + [(1, d) for d in range(16)] + [(2, d) for d in range(16)]
          + [(0, 16), (0, 17), (1, 16), (1, 17), (2, 16), (2, 17), None, None])


def _row_tile(j):
    return pl.multiple_of(jnp.minimum(j * 128, D - 128), 64)


def _ln_stats(x):
    m = jnp.mean(x, axis=0, keepdims=True)
    xc = x - m
    v = jnp.mean(xc * xc, axis=0, keepdims=True)
    r = jax.lax.rsqrt(v + EPS)
    return m, r, xc * r


def _head_reduce(p):
    p = p + pltpu.roll(p, 64, 1)
    return p + pltpu.roll(p, 32, 1)


def kernel(xT_hbm, gT_hbm, wqkv_hbm, wo_hbm, w1_ref, b1_ref, w2T_ref, b2_ref,
           outT_hbm, dxT_hbm, dwqkv_hbm, dwo_hbm, dw1_ref, db1_ref, dw2T_ref, db2_ref,
           xT_s, gT_s, wqkv_s, wo_s, outT_s, dxT_s, dwqkv_s, dwo_s, dwo_t,
           xnT_s, yT_s, y_s, g_s, stats_s, wq_s, woT_s, tmp_s, tmp2_s,
           Q_s, K_s, V_s, DO_s, A_s, DL_s, dqkv_s, o_s, oacc_s, dyacc_s, dwq_s, dwoT_s,
           sem_in, sem_out):
    c = pl.program_id(0)

    def in_copy(src, dst, j, k):
        cols = pl.ds(pl.multiple_of(j * TB, TB), TB)
        return pltpu.make_async_copy(src.at[:, cols], dst.at[:, cols], sem_in.at[k, j])

    def out_copy(src, dst, j, k):
        cols = pl.ds(pl.multiple_of(j * TB, TB), TB)
        return pltpu.make_async_copy(src.at[:, cols], dst.at[:, cols], sem_out.at[k, j])

    wo_copy = pltpu.make_async_copy(wo_hbm, wo_s, sem_in.at[2, 0])
    wqkv_copy = pltpu.make_async_copy(wqkv_hbm, wqkv_s, sem_in.at[2, 1])
    dwo_copy = pltpu.make_async_copy(dwo_s, dwo_hbm, sem_out.at[2, 0])
    dwqkv_copy = pltpu.make_async_copy(dwqkv_s.at[pl.ds(0, D), :], dwqkv_hbm, sem_out.at[2, 1])

    def _prologue():
        wo_copy.start()
        wqkv_copy.start()
        for j in range(NB):
            in_copy(xT_hbm, xT_s, j, 0).start()
            in_copy(gT_hbm, gT_s, j, 1).start()
        lane16 = jax.lax.broadcasted_iota(jnp.int32, (PAD, 128), 1)
        z = jnp.zeros((PAD, 128), f32)
        for t in range(5):
            K_s[t, pl.ds(0, PAD), :] = z if t < 4 else jnp.where((lane16 >= 64) & (lane16 < 96), NEG, 0.0)
            V_s[t, pl.ds(0, PAD), :] = z
            Q_s[t, pl.ds(S, PAD), :] = z
            DO_s[t, pl.ds(S, PAD), :] = z
        for w in range(W):
            A_s[w, pl.ds(S, PAD), :] = z
            DL_s[w, pl.ds(S, PAD), :] = z
        dwoT_s[pl.ds(D, DP - D), :] = jnp.zeros((DP - D, DP), f32)
        wo_copy.wait()
        b2row = b2_ref[...].astype(f32).reshape(1, D)
        for j in range(5):
            wd = 128 if j < 4 else 64
            if j == 4:
                tmp_s[pl.ds(0, D), :] = jnp.zeros((D, 128), f32)
            tmp_s[pl.ds(0, D), pl.ds(0, wd)] = wo_s[:, pl.ds(j * 128, wd)].astype(f32)
            parts = [tmp_s[pl.ds(d, 32, stride=DH), :] for d in range(DH)]
            brow = b2row[:, j * 128:j * 128 + wd]
            if wd < 128:
                brow = jnp.concatenate([brow, jnp.zeros((1, 128 - wd), f32)], axis=1)
            row = jax.lax.broadcasted_iota(jnp.int32, (64, 128), 0)
            parts.append(jnp.where(row == 0, jnp.broadcast_to(brow, (64, 128)), 0.0))
            blk = jnp.concatenate(parts, axis=0).T.astype(bf16)
            woT_s[pl.ds(j * 128, wd), :] = blk[:wd]
        wqkv_copy.wait()

        def perm_body(j, carry):
            r0 = _row_tile(j)
            tmp_s[pl.ds(0, 3 * D), :] = wqkv_s[pl.ds(r0, 128), :].astype(f32).T
            parts = []
            for grp in GROUPS:
                if grp is None:
                    parts.append(jnp.zeros((32, 128), f32))
                else:
                    t, d = grp
                    parts.append(tmp_s[pl.ds(t * D + d, 32, stride=DH), :])
            wq_s[pl.ds(r0, 128), :] = jnp.concatenate(parts, axis=0).T.astype(bf16)
            return carry

        jax.lax.fori_loop(0, 5, perm_body, 0)

        laneb = jax.lax.broadcasted_iota(jnp.int32, (TB, 128), 1)

        def blk_body(j, carry):
            in_copy(xT_hbm, xT_s, j, 0).wait()
            in_copy(gT_hbm, gT_s, j, 1).wait()
            c0 = pl.multiple_of(j * TB, TB)
            cols = pl.ds(c0, TB)
            x = xT_s[:, cols].astype(f32)
            m1, r1, xn = _ln_stats(x)
            m2, r2, y = _ln_stats(xn)
            stats_s[0:1, cols] = m1
            stats_s[1:2, cols] = r1
            stats_s[2:3, cols] = m2
            stats_s[3:4, cols] = r2
            xnb = xn.astype(bf16)
            yb = y.astype(bf16)
            xnT_s[:, cols] = xnb
            yT_s[:, cols] = yb
            y_s[cols, :] = yb.T
            gb = gT_s[:, cols].T
            g_s[cols, :] = gb
            oacc_s[:, cols] = x
            dyacc_s[:, cols] = jnp.zeros((D, TB), f32)
            qkv = NN(xnb.T, wq_s[...])
            krows = pl.ds(c0 + PAD, TB)
            for t in range(4):
                Q_s[t, cols, :] = qkv[:, t * 128:(t + 1) * 128] * SCALE
                K_s[t, krows, :] = qkv[:, (4 + t) * 128:(5 + t) * 128]
                V_s[t, krows, :] = qkv[:, (8 + t) * 128:(9 + t) * 128]
            t12 = qkv[:, 12 * 128:13 * 128]
            Q_s[4, cols, :] = jnp.where(laneb < 64, t12 * SCALE, jnp.where(laneb < 96, 1.0, 0.0))
            K_s[4, krows, :] = jnp.where(laneb < 64, pltpu.roll(t12, 64, 1), 0.0)
            V_s[4, krows, :] = qkv[:, 13 * 128:14 * 128]
            do = NN(gb, woT_s[...])
            for t in range(5):
                DO_s[t, cols, :] = do[:, t * 128:(t + 1) * 128]
            return carry

        with jax.named_scope('blk_loop'):
            jax.lax.fori_loop(0, NB, blk_body, 0)

    with jax.named_scope('prologue'):
        pl.when(c == 0)(_prologue)

    lane = jax.lax.broadcasted_iota(jnp.int32, (RA, 128), 1)

    def attn_rows(r):
        rows = pl.ds(r, RA)
        q = [Q_s[t, rows, :] for t in range(5)]
        do = [DO_s[t, rows, :] for t in range(5)]
        lg, da = [], []
        for w in range(W):
            kr = pl.ds(r + PAD - DIL * w, RA)
            p = q[0] * K_s[0, kr, :]
            pd = do[0] * V_s[0, kr, :]
            for t in range(1, 5):
                p = p + q[t] * K_s[t, kr, :]
                pd = pd + do[t] * V_s[t, kr, :]
            lg.append(_head_reduce(p))
            da.append(_head_reduce(pd))
        m = functools.reduce(jnp.maximum, lg)
        e = [jnp.exp(l - m) for l in lg]
        inv = 1.0 / functools.reduce(jnp.add, e)
        a = [x * inv for x in e]
        cc = functools.reduce(jnp.add, [a[w] * da[w] for w in range(W)])
        dl = [a[w] * (da[w] - cc) for w in range(W)]
        for w in range(W):
            A_s[w, rows, :] = a[w]
            DL_s[w, rows, :] = dl[w]
        dq4 = None
        for t in range(5):
            o = None
            dq = None
            for w in range(W):
                kr = pl.ds(r + PAD - DIL * w, RA)
                vo = a[w] * V_s[t, kr, :]
                vq = dl[w] * K_s[t, kr, :]
                o = vo if o is None else o + vo
                dq = vq if dq is None else dq + vq
            dq = dq * SCALE
            if t < 4:
                o_s[rows, t * 128:(t + 1) * 128] = o.astype(bf16)
                dqkv_s[rows, t * 128:(t + 1) * 128] = dq.astype(bf16)
            else:
                o_s[rows, 512:640] = jnp.where(lane == 64, 1.0, o).astype(bf16)
                dq4 = dq
        af = [A_s[w, pl.ds(r + DIL * w, RA), :] for w in range(W)]
        df = [DL_s[w, pl.ds(r + DIL * w, RA), :] for w in range(W)]
        for t in range(5):
            dk = None
            dv = None
            for w in range(W):
                fr = pl.ds(r + DIL * w, RA)
                vk = df[w] * Q_s[t, fr, :]
                vv = af[w] * DO_s[t, fr, :]
                dk = vk if dk is None else dk + vk
                dv = vv if dv is None else dv + vv
            if t < 4:
                dqkv_s[rows, (4 + t) * 128:(5 + t) * 128] = dk.astype(bf16)
                dqkv_s[rows, (8 + t) * 128:(9 + t) * 128] = dv.astype(bf16)
            else:
                dqkv_s[rows, 12 * 128:13 * 128] = jnp.where(lane < 64, dq4, pltpu.roll(dk, 64, 1)).astype(bf16)
                dqkv_s[rows, 13 * 128:14 * 128] = jnp.where(lane < 64, dv, 0.0).astype(bf16)

    with jax.named_scope('mlp'):
        rs0 = pl.multiple_of(jnp.maximum(S - RS - c * RS, 0), RS)
        for b in reversed(range(RS // RA)):
            attn_rows(pl.multiple_of(rs0 + b * RA, RA))

        w1c = w1_ref[...]
        w2c = w2T_ref[...]
        b1c = b1_ref[...].astype(f32).reshape(1, TF)
        hpre = NN(y_s[...], w1c) + b1c
        dh = NN(g_s[...], w2c)
        x2 = hpre * hpre
        t = jnp.tanh(hpre * (C0 + (C0 * C1) * x2))
        hx = 0.5 * hpre
        opt = 1.0 + t
        hb = (hx * opt).astype(bf16)
        gp = 0.5 * opt + hx * (1.0 - t * t) * (C0 + (3 * C0 * C1) * x2)
        dhp = dh * gp
        db1_ref[...] = jnp.sum(dhp, axis=0).astype(bf16)
        dhb = dhp.astype(bf16)
        oacc_s[...] += NT(w2c, hb)
        dyacc_s[...] += NT(w1c, dhb)
        dw2T_ref[...] = NN(gT_s[...], hb).astype(bf16)
        dw1_ref[...] = NN(yT_s[...], dhb).astype(bf16)

    def _tail():
        def dwo_body(n, carry):
            cols = pl.ds(pl.multiple_of(n * 128, 128), 128)
            dwoT_s[pl.ds(0, D), cols] = NN(gT_s[...], o_s[:, cols])
            return carry

        with jax.named_scope('dwo_loop'):
            jax.lax.fori_loop(0, 5, dwo_body, 0)

        def dwq_body(n, carry):
            cols = pl.ds(pl.multiple_of(n * 256, 256), 256)
            dwq_s[:, cols] = NN(xnT_s[...], dqkv_s[:, cols])
            jt = jnp.minimum(n, 4)
            r0 = pl.multiple_of(jt * 128, 128)
            blk = dwoT_s[pl.ds(r0, 128), :].T
            for d in range(DH):
                tmp_s[pl.ds(d, 32, stride=DH), :] = blk[d * 32:(d + 1) * 32, :]
            dwo_t[:, pl.ds(r0, 128)] = tmp_s[pl.ds(0, D), :].astype(bf16)
            tmp2_s[:, pl.ds(r0, 128)] = blk[D:D + 8, :]
            return carry

        with jax.named_scope('dwq_loop'):
            jax.lax.fori_loop(0, NQ // 2, dwq_body, 0)
        db2_ref[...] = tmp2_s[0:1, 0:D].reshape(D).astype(bf16)
        dwo_s[...] = dwo_t[:, 0:D]
        dwo_copy.start()

        def fin_body(j, carry):
            c0 = pl.multiple_of(j * TB, TB)
            cols = pl.ds(c0, TB)
            outT_s[:, cols] = (oacc_s[:, cols] + NT(woT_s[...], o_s[cols, :])).astype(bf16)
            m1 = stats_s[0:1, cols]
            r1 = stats_s[1:2, cols]
            m2 = stats_s[2:3, cols]
            r2 = stats_s[3:4, cols]
            xn = (xT_s[:, cols].astype(f32) - m1) * r1
            y = (xn - m2) * r2
            dy = dyacc_s[:, cols]
            dxn = r2 * (dy - jnp.mean(dy, axis=0, keepdims=True) - y * jnp.mean(dy * y, axis=0, keepdims=True))
            dxn = dxn + NT(wq_s[...], dqkv_s[cols, :])
            dx = r1 * (dxn - jnp.mean(dxn, axis=0, keepdims=True) - xn * jnp.mean(dxn * xn, axis=0, keepdims=True))
            dxT_s[:, cols] = (gT_s[:, cols].astype(f32) + dx).astype(bf16)
            r0 = _row_tile(j)
            rd = pl.multiple_of(jnp.where(j < 5, r0, D), 64)
            blk = dwq_s[pl.ds(r0, 128), :].T
            for gi, grp in enumerate(GROUPS):
                if grp is None:
                    continue
                tt, d = grp
                tmp_s[pl.ds(tt * D + d, 32, stride=DH), :] = blk[gi * 32:(gi + 1) * 32, :]
            dwqkv_s[pl.ds(rd, 128), :] = tmp_s[pl.ds(0, 3 * D), :].T.astype(bf16)
            out_copy(outT_s, outT_hbm, j, 0).start()
            out_copy(dxT_s, dxT_hbm, j, 1).start()

            @pl.when(j == 4)
            def _():
                dwqkv_copy.start()
            return carry

        with jax.named_scope('fin_loop'):
            jax.lax.fori_loop(0, NB, fin_body, 0)
        dwo_copy.wait()
        dwqkv_copy.wait()
        for j in range(NB):
            out_copy(outT_s, outT_hbm, j, 0).wait()
            out_copy(dxT_s, dxT_hbm, j, 1).wait()

    with jax.named_scope('tail'):
        pl.when(c == NF - 1)(_tail)


def _full(shape):
    return pl.BlockSpec(shape, lambda c: (0,) * len(shape))


@jax.jit
def pallas_parallel_sum__sliding_local_dilated__mixer_channel_mlp__prompt_kernel(A_x, A_wqkv, A_wo, B_x, B_w1, B_b1, B_w2, B_b2, grad_out):
    xT = A_x.reshape(S, D).T
    gT = grad_out.reshape(S, D).T
    w2T = B_w2.T
    anyspec = pl.BlockSpec(memory_space=pl.ANY)
    outs = pl.pallas_call(
        kernel,
        grid=(NF,),
        in_specs=[anyspec, anyspec, anyspec, anyspec,
                  pl.BlockSpec((D, TF), lambda c: (0, c)),
                  pl.BlockSpec((TF,), lambda c: (c,)),
                  pl.BlockSpec((D, TF), lambda c: (0, c)),
                  _full((D,))],
        out_specs=[anyspec, anyspec, anyspec, anyspec,
                   pl.BlockSpec((D, TF), lambda c: (0, c)),
                   pl.BlockSpec((TF,), lambda c: (c,)),
                   pl.BlockSpec((D, TF), lambda c: (0, c)),
                   _full((D,))],
        out_shape=[jax.ShapeDtypeStruct((D, S), bf16), jax.ShapeDtypeStruct((D, S), bf16),
                   jax.ShapeDtypeStruct((D, 3 * D), bf16), jax.ShapeDtypeStruct((D, D), bf16),
                   jax.ShapeDtypeStruct((D, F), bf16), jax.ShapeDtypeStruct((F,), bf16),
                   jax.ShapeDtypeStruct((D, F), bf16), jax.ShapeDtypeStruct((D,), bf16)],
        scratch_shapes=[
            pltpu.VMEM((D, S), bf16),
            pltpu.VMEM((D, S), bf16),
            pltpu.VMEM((D, 3 * D), bf16),
            pltpu.VMEM((D, D), bf16),
            pltpu.VMEM((D, S), bf16),
            pltpu.VMEM((D, S), bf16),
            pltpu.VMEM((D + 128, 3 * D), bf16),
            pltpu.VMEM((D, D), bf16),
            pltpu.VMEM((D, DP), bf16),
            pltpu.VMEM((D, S), bf16),
            pltpu.VMEM((D, S), bf16),
            pltpu.VMEM((S, D), bf16),
            pltpu.VMEM((S, D), bf16),
            pltpu.VMEM((8, S), f32),
            pltpu.VMEM((D, QP), bf16),
            pltpu.VMEM((D, DP), bf16),
            pltpu.VMEM((QP, 128), f32),
            pltpu.VMEM((8, DP), f32),
            pltpu.VMEM((5, S + PAD, 128), f32),
            pltpu.VMEM((5, S + PAD, 128), f32),
            pltpu.VMEM((5, S + PAD, 128), f32),
            pltpu.VMEM((5, S + PAD, 128), f32),
            pltpu.VMEM((W, S + PAD, 128), f32),
            pltpu.VMEM((W, S + PAD, 128), f32),
            pltpu.VMEM((S, QP), bf16),
            pltpu.VMEM((S, DP), bf16),
            pltpu.VMEM((D, S), f32),
            pltpu.VMEM((D, S), f32),
            pltpu.VMEM((D, QP), f32),
            pltpu.VMEM((DP, DP), f32),
            pltpu.SemaphoreType.DMA((3, NB)),
            pltpu.SemaphoreType.DMA((3, NB)),
        ],
        compiler_params=pltpu.CompilerParams(dimension_semantics=("arbitrary",),
                                             vmem_limit_bytes=120 * 1024 * 1024),
    )(xT, gT, A_wqkv, A_wo, B_w1, B_b1, w2T, B_b2)
    outT, dxT, dwqkv, dwo, dw1, db1, dw2T, db2 = outs
    return (outT.T.reshape(1, S, D), dxT.T.reshape(1, S, D), dwqkv, dwo, dw1, db1, dw2T.T, db2)
```

```python
import functools
import os
import jax
import jax.numpy as jnp
import jax.experimental.pallas as pl
import jax.experimental.pallas.tpu as pltpu

S, D, F = 2048, 576, 4608
H, DH, W, DIL = 32, 18, 8, 2
DP = 640
NQ = 14
QP = NQ * 128
PAD = 16
EPS = 1e-5
SCALE = DH ** -0.5
C0 = 0.7978845608028654
C1 = 0.044715
NEG = -1e9

TF = 256
NF = F // TF
TB = 256
NB = S // TB
RA = 8
RS = 128
NSL = S // RS
NOSER = int(os.environ.get('NOSER', 2))

f32 = jnp.float32
bf16 = jnp.bfloat16


def NN(a, b):
    return jax.lax.dot_general(a, b, (((1,), (0,)), ((), ())), preferred_element_type=f32)


def NT(a, b):
    return jax.lax.dot_general(a, b, (((1,), (1,)), ((), ())), preferred_element_type=f32)


GROUPS = ([(0, d) for d in range(16)] + [(1, d) for d in range(16)] + [(2, d) for d in range(16)]
          + [(2, 16), (2, 17), (1, 16), (1, 17), None, None, (0, 16), (0, 17)])
WQ_PIECES = ((0, 128), (128, 128), (256, 128), (384, 192))


def _row_tile(j):
    return pl.multiple_of(jnp.minimum(j * 128, D - 128), 64)


def _colmean(x):
    return jnp.sum(x, axis=0, keepdims=True) * (1.0 / D)


def _head_reduce(p):
    p = p + pltpu.roll(p, 64, 1)
    return p + pltpu.roll(p, 32, 1)


def kernel(xT_hbm, gT_hbm, wqkv_hbm, wo_hbm, w1_hbm, b1_hbm, w2T_hbm, b2_hbm,
           outT_hbm, dxT_hbm, dwqkv_hbm, dwo_hbm, dw1_hbm, db1_hbm, dw2T_hbm, db2_hbm,
           b1_ref, b2_ref, db1_ref, db2_ref,
           xT_s, gT_s, wqkv_s, wo_s, w1_s, w2T_s, dw1_s, dw2T_s, dwqkv_s, dwo_s, dwo_t,
           xnT_s, yT_s, xn_s, y_s, g_s, stats_s, wq_s, woT_s, tmp_s, tmp2_s,
           P_s, dqkv_s, o_s, oacc_s, dyacc_s, dwq_s, dwoT_s, dxn_s,
           WK, WV, WQ, WDO, WA, WDL,
           sem_in, sem_out, sem_dw):
    outT_s = xnT_s
    dxT_s = yT_s

    def blk(j):
        return pl.ds(pl.multiple_of(j * TB, TB), TB)

    def in_copy(src, dst, j, k):
        return pltpu.make_async_copy(src.at[:, blk(j)], dst.at[:, blk(j)], sem_in.at[k, j])

    def out_copy(src, dst, j, k):
        return pltpu.make_async_copy(src.at[:, blk(j)], dst.at[:, blk(j)], sem_out.at[k, j])

    def wqkv_copy(i):
        r0, n = WQ_PIECES[i]
        return pltpu.make_async_copy(wqkv_hbm.at[pl.ds(r0, n), :], wqkv_s.at[pl.ds(r0, n), :], sem_in.at[2, 1 + i])

    def chunk(c):
        return pl.ds(pl.multiple_of(c * TF, TF), TF)

    def dw_copy(src, dst, c, k):
        return pltpu.make_async_copy(src.at[:, chunk(c)], dst.at[:, chunk(c)], sem_dw.at[k, c])

    b1_copy = pltpu.make_async_copy(b1_hbm, b1_ref, sem_in.at[2, 7])
    b2_copy = pltpu.make_async_copy(b2_hbm, b2_ref, sem_in.at[3, 0])
    db1_copy = pltpu.make_async_copy(db1_ref, db1_hbm, sem_out.at[2, 2])
    db2_copy = pltpu.make_async_copy(db2_ref, db2_hbm, sem_out.at[2, 3])
    w1_copy = pltpu.make_async_copy(w1_hbm, w1_s, sem_in.at[2, 5])
    w2_copy = pltpu.make_async_copy(w2T_hbm, w2T_s, sem_in.at[2, 6])
    wo_copy = pltpu.make_async_copy(wo_hbm, wo_s, sem_in.at[2, 0])
    dwo_copy = pltpu.make_async_copy(dwo_s, dwo_hbm, sem_out.at[2, 0])
    dwqkv_copy = pltpu.make_async_copy(dwqkv_s.at[pl.ds(0, D), :], dwqkv_hbm, sem_out.at[2, 1])

    def ln_block(j):
        cols = blk(j)
        x = xT_s[:, cols].astype(f32)
        m1 = _colmean(x)
        xc = x - m1
        v1 = _colmean(xc * xc)
        r1 = jax.lax.rsqrt(v1 + EPS)
        v2 = v1 * r1 * r1
        r2 = jax.lax.rsqrt(v2 + EPS)
        stats_s[0:1, cols] = m1
        stats_s[1:2, cols] = r1
        stats_s[2:3, cols] = v2
        stats_s[3:4, cols] = r2
        xnb = (xc * r1).astype(bf16)
        yb = (xc * (r1 * r2)).astype(bf16)
        xnT_s[:, cols] = xnb
        yT_s[:, cols] = yb
        xn_s[cols, :] = xnb.T
        y_s[cols, :] = yb.T

    def _prologue():
        b2_copy.start()
        wo_copy.start()
        in_copy(gT_hbm, gT_s, 0, 1).start()
        for i in range(4):
            in_copy(gT_hbm, gT_s, i + 1, 1).start()
            wqkv_copy(i).start()
        for j in range(5, NB):
            in_copy(gT_hbm, gT_s, j, 1).start()
        for j in range(NB):
            in_copy(xT_hbm, xT_s, j, 0).start()
        w1_copy.start()
        w2_copy.start()
        b1_copy.start()
        for t in range(NQ):
            P_s[t, pl.ds(0, PAD), :] = jnp.zeros((PAD, 128), f32)
        dwoT_s[pl.ds(D, DP - D), :] = jnp.zeros((DP - D, DP), f32)
        zw = jnp.zeros((RS + PAD, 128), f32)
        for w in range(W):
            WA[w, pl.ds(0, RS + PAD), :] = zw
            WDL[w, pl.ds(0, RS + PAD), :] = zw
        for t in (0, 1, 2, 3, 5):
            WQ[t, pl.ds(0, RS + PAD), :] = zw
        for t in range(4):
            WDO[t, pl.ds(0, RS + PAD), :] = zw
        wo_copy.wait()
        b2_copy.wait()
        b2row = b2_ref[...].astype(f32).reshape(1, D)
        for j in range(5):
            wd = 128 if j < 4 else 64
            base = (j % 2) * D
            if j == 4:
                tmp_s[pl.ds(base, D), :] = jnp.zeros((D, 128), f32)
            tmp_s[pl.ds(base, D), pl.ds(0, wd)] = wo_s[:, pl.ds(j * 128, wd)].astype(f32)
            parts = [tmp_s[pl.ds(base + d, 32, stride=DH), :] for d in range(DH)]
            brow = b2row[:, j * 128:j * 128 + wd]
            if wd < 128:
                brow = jnp.concatenate([brow, jnp.zeros((1, 128 - wd), f32)], axis=1)
            row = jax.lax.broadcasted_iota(jnp.int32, (64, 128), 0)
            parts.append(jnp.where(row == 0, jnp.broadcast_to(brow, (64, 128)), 0.0))
            wblk = jnp.concatenate(parts, axis=0).astype(bf16).T
            woT_s[pl.ds(j * 128, wd), :] = wblk[:wd]

        in_copy(gT_hbm, gT_s, 0, 1).wait()
        g_s[blk(0), :] = gT_s[:, blk(0)].T

        def do_block(j):
            jn = jnp.minimum(j + 1, NB - 1)
            do = NN(g_s[blk(j), :], woT_s[...])
            g_s[blk(jn), :] = gT_s[:, blk(jn)].T
            prow = pl.ds(pl.multiple_of(j * TB + PAD, PAD), TB)
            for t in range(5):
                P_s[NQ + t, prow, :] = do[:, t * 128:(t + 1) * 128]

        def p2a_body(j, carry):
            in_copy(gT_hbm, gT_s, j + 1, 1).wait()
            for i in range(4):
                @pl.when(j == i)
                def _():
                    wqkv_copy(i).wait()
            do_block(j)
            r0 = _row_tile(j)
            tmp_s[pl.ds(0, 3 * D), :] = wqkv_s[pl.ds(r0, 128), :].T.astype(f32)
            parts = []
            for grp in GROUPS:
                if grp is None:
                    parts.append(jnp.zeros((32, 128), f32))
                else:
                    t, d = grp
                    parts.append(tmp_s[pl.ds(t * D + d, 32, stride=DH), :])
            wq_s[pl.ds(r0, 128), :] = jnp.concatenate(parts, axis=0).astype(bf16).T
            return carry

        def p2b_body(j, carry):
            @pl.when(j < NB - 1)
            def _():
                in_copy(gT_hbm, gT_s, jnp.minimum(j + 1, NB - 1), 1).wait()
            in_copy(xT_hbm, xT_s, j - 5, 0).wait()
            do_block(j)
            ln_block(j - 5)
            return carry

        with jax.named_scope('p2_loop'):
            jax.lax.fori_loop(0, 5, p2a_body, 0)
            jax.lax.fori_loop(5, NB, p2b_body, 0)

        def p3_body(j, carry):
            jn = jnp.minimum(j + 3, NB - 1)

            @pl.when(j + 3 < NB)
            def _():
                in_copy(xT_hbm, xT_s, jn, 0).wait()
            qkv = NN(xn_s[blk(j), :], wq_s[...])
            prow = pl.ds(pl.multiple_of(j * TB + PAD, PAD), TB)
            for t in range(NQ):
                P_s[t, prow, :] = qkv[:, t * 128:(t + 1) * 128]
            ln_block(jn)
            return carry

        with jax.named_scope('p3_loop'):
            jax.lax.fori_loop(0, NB, p3_body, 0)

    with jax.named_scope('prologue'):
        _prologue()
        w1_copy.wait()
        w2_copy.wait()
        b1_copy.wait()

    lane = jax.lax.broadcasted_iota(jnp.int32, (RA, 128), 1)

    def chain(ms, load, prev):
        acc = None
        for w in range(W):
            v = ms[w] * load(w)
            if acc is None:
                acc = v if prev is None else v + prev * 0.0
            else:
                acc = acc + v
        return acc

    def attn_a2(rs, lr, ser):
        rows = pl.ds(rs + lr, RA)
        lrows = pl.ds(lr, RA)
        kr = lambda w: pl.ds(lr + PAD - DIL * w, RA)
        q = [WQ[t, lrows, :] for t in range(5)]
        do = [WDO[t, lrows, :] for t in range(5)]
        lg, da = [], []
        for w in range(W):
            p = q[0] * WK[0, kr(w), :]
            pd = do[0] * WV[0, kr(w), :]
            for t in range(1, 5):
                p = p + q[t] * WK[t, kr(w), :]
                pd = pd + do[t] * WV[t, kr(w), :]
            lg.append(_head_reduce(p))
            da.append(_head_reduce(pd))
        m = functools.reduce(jnp.maximum, lg)
        e = [jnp.exp(l - m) for l in lg]
        inv = 1.0 / functools.reduce(jnp.add, e)
        a = [x * inv for x in e]
        cc = functools.reduce(jnp.add, [a[w] * da[w] for w in range(W)])
        dl = [a[w] * (da[w] - cc) for w in range(W)]
        for w in range(W):
            WA[w, lrows, :] = a[w]
            WDL[w, lrows, :] = dl[w]
        prev = None
        for t in range(4):
            o = chain(a, lambda w: WV[t, kr(w), :], prev)
            o_s[rows, t * 128:(t + 1) * 128] = o.astype(bf16)
            dq = chain(dl, lambda w: WK[t, kr(w), :], o if ser else None)
            dqkv_s[rows, t * 128:(t + 1) * 128] = (dq * SCALE).astype(bf16)
            prev = dq if ser else None
        mix = [jnp.where(lane < 64, a[w], dl[w]) for w in range(W)]
        acc = chain(mix, lambda w: WV[4, kr(w), :], prev)
        o_s[rows, 512:640] = jnp.where(lane < 64, acc, jnp.where(lane == 64, 1.0, 0.0)).astype(bf16)
        dqkv_s[rows, 13 * 128:14 * 128] = jnp.where(lane < 64, 0.0, acc * SCALE).astype(bf16)

    def attn_a3(rs, lr, prev):
        rows = pl.ds(rs + lr, RA)
        fr = lambda w: pl.ds(RS + lr + DIL * w, RA)
        af = [WA[w, fr(w), :] for w in range(W)]
        df = [WDL[w, fr(w), :] for w in range(W)]
        for t in range(4):
            dk = chain(df, lambda w: WQ[t, fr(w), :], prev)
            dqkv_s[rows, (4 + t) * 128:(5 + t) * 128] = dk.astype(bf16)
            dv = chain(af, lambda w: WDO[t, fr(w), :], dk)
            dqkv_s[rows, (8 + t) * 128:(9 + t) * 128] = dv.astype(bf16)
            prev = dv
        mix = [jnp.where(lane < 64, af[w], df[w]) for w in range(W)]
        acc = chain(mix, lambda w: WQ[5, fr(w), :], prev)
        dqkv_s[rows, 12 * 128:13 * 128] = acc.astype(bf16)
        return acc

    def attn_slice(c):
        rs0 = pl.multiple_of(jnp.maximum(NSL - 1 - c, 0) * RS, RS)
        rs1 = pl.multiple_of(jnp.where((c >= 1) & (c <= NSL), NSL - c, NSL) * RS, RS)
        hi = pl.ds(RS, RS + PAD)
        lo = pl.ds(0, RS + PAD)
        cur = pl.ds(0, RS)
        for w in range(W):
            WA[w, hi, :] = WA[w, lo, :]
            WDL[w, hi, :] = WDL[w, lo, :]
        for t in (0, 1, 2, 3, 5):
            WQ[t, hi, :] = WQ[t, lo, :]
        for t in range(4):
            WDO[t, hi, :] = WDO[t, lo, :]
        src = pl.ds(rs0 + PAD, RS)
        srch = pl.ds(rs0, RS + PAD)
        for t in range(4):
            WQ[t, cur, :] = P_s[t, src, :] * SCALE
            WDO[t, cur, :] = P_s[NQ + t, src, :]
            WK[t] = P_s[4 + t, srch, :]
            WV[t] = P_s[8 + t, srch, :]
        ln = jax.lax.broadcasted_iota(jnp.int32, (RS, 128), 1)
        q4 = P_s[13, src, :] * SCALE
        do4 = jnp.where(ln < 64, P_s[NQ + 4, src, :], 0.0)
        WQ[4, cur, :] = jnp.where(ln < 32, 1.0, q4)
        WQ[5, cur, :] = do4 + q4
        WDO[4, cur, :] = do4
        lnh = jax.lax.broadcasted_iota(jnp.int32, (RS + PAD, 128), 1)
        rowh = jax.lax.broadcasted_iota(jnp.int32, (RS + PAD, 128), 0) + rs0
        t12 = P_s[12, srch, :]
        WV[4] = t12
        WK[4] = jnp.where(lnh < 64, jnp.where((lnh < 32) & (rowh < PAD), NEG, 0.0), t12)
        p = None
        for b in reversed(range(RS // RA)):
            p = attn_a3(rs1, b * RA, p)
        for b in reversed(range(RS // RA)):
            attn_a2(rs0, b * RA, b >= NOSER)

    def mlp_body(c, carry):
        attn_slice(c)
        ck = chunk(c)
        w1c = w1_s[:, ck]
        w2c = w2T_s[:, ck]
        b1c = b1_ref[ck].astype(f32).reshape(1, TF)
        hpre = NN(y_s[...], w1c) + b1c
        dh = NN(g_s[...], w2c)
        x2 = hpre * hpre
        t = jnp.tanh(hpre * (C0 + (C0 * C1) * x2))
        hx = 0.5 * hpre
        opt = 1.0 + t
        hb = (hx * opt).astype(bf16)
        gp = 0.5 * opt + hx * (1.0 - t * t) * (C0 + (3 * C0 * C1) * x2)
        dhp = dh * gp
        db1_ref[ck] = jnp.sum(dhp, axis=0).astype(bf16)
        dhb = dhp.astype(bf16)
        oacc_s[...] = jnp.where(c > 0, oacc_s[...], 0.0) + NT(w2c, hb)
        dyacc_s[...] = jnp.where(c > 0, dyacc_s[...], 0.0) + NT(w1c, dhb)
        dw2T_s[:, ck] = NN(gT_s[...], hb).astype(bf16)
        dw1_s[:, ck] = NN(yT_s[...], dhb).astype(bf16)
        dw_copy(dw1_s, dw1_hbm, c, 0).start()
        dw_copy(dw2T_s, dw2T_hbm, c, 1).start()
        return carry

    with jax.named_scope('mlp'):
        jax.lax.fori_loop(0, NF, mlp_body, 0)

    def _tail():
        db1_copy.start()
        def dwo_body(n, carry):
            cols = pl.ds(pl.multiple_of(n * 128, 128), 128)
            dwoT_s[pl.ds(0, D), cols] = NN(gT_s[...], o_s[:, cols])
            return carry

        with jax.named_scope('dwo_loop'):
            jax.lax.fori_loop(0, 5, dwo_body, 0)

        def dwq_body(n, carry):
            cols = pl.ds(pl.multiple_of(n * 256, 256), 256)
            dwq_s[:, cols] = NN(xnT_s[...], dqkv_s[pl.ds(0, S), cols])
            jt = jnp.minimum(n, 4)
            r0 = pl.multiple_of(jt * 128, 128)
            tb = dwoT_s[pl.ds(r0, 128), :].T
            for d in range(DH):
                tmp_s[pl.ds(d, 32, stride=DH), :] = tb[d * 32:(d + 1) * 32, :]
            dwo_t[:, pl.ds(r0, 128)] = tmp_s[pl.ds(0, D), :].astype(bf16)
            tmp2_s[:, pl.ds(r0, 128)] = tb[D:D + 8, :]
            return carry

        with jax.named_scope('dwq_loop'):
            jax.lax.fori_loop(0, NQ // 2, dwq_body, 0)
        db2_ref[...] = tmp2_s[0:1, 0:D].reshape(D).astype(bf16)
        dwo_s[...] = dwo_t[:, 0:D]
        dwo_copy.start()
        db2_copy.start()

        def fin_dx(j, thin):
            RC = 16
            bc = lambda v: jnp.broadcast_to(v, (RC, 128))
            red = lambda v: jnp.sum(v, axis=0, keepdims=True) * (1.0 / D)
            link = None
            for h in range(TB // 128):
                if os.environ.get('HL', '0') == '0':
                    link = None
                cols = pl.ds(pl.multiple_of(j * TB + h * 128, 128), 128)
                lc = pl.ds(h * 128, 128)
                m1 = stats_s[0:1, cols]
                r1 = stats_s[1:2, cols]
                v2 = stats_s[2:3, cols]
                r2 = stats_s[3:4, cols]
                m1b, r1b, r2b = bc(m1), bc(r1), bc(r2)
                su = sux = sb = None
                for k in range(D // RC):
                    rr = pl.ds(k * RC, RC)
                    mk = m1b if (link is None or not thin) else m1b + link * 0.0
                    xn = (xT_s[rr, cols].astype(f32) - mk) * r1b
                    dy = dyacc_s[rr, cols]
                    u = dxn_s[rr, lc] + r2b * dy
                    su = u if su is None else su + u
                    sux = u * xn if sux is None else sux + u * xn
                    sb = dy * xn if sb is None else sb + dy * xn
                    link = sux
                k0 = bc(red(su))
                k1 = bc(red(sux) + (r2 * r2 * r2) * (1.0 - v2) * red(sb))
                for k in range(D // RC):
                    rr = pl.ds(k * RC, RC)
                    mk = m1b if not thin else m1b + link * 0.0
                    xn = (xT_s[rr, cols].astype(f32) - mk) * r1b
                    u = dxn_s[rr, lc] + r2b * dyacc_s[rr, cols]
                    dx = r1b * (u - k0 - xn * k1)
                    dxT_s[rr, cols] = (gT_s[rr, cols].astype(f32) + dx).astype(bf16)
                    link = dx
            return link

        def fin_body(j, carry):
            cols = blk(j)
            dxn_s[...] = NT(wq_s[...], dqkv_s[cols, :])
            outT_s[:, cols] = (oacc_s[:, cols] + xT_s[:, cols].astype(f32) + NT(woT_s[...], o_s[cols, :])).astype(bf16)
            link = fin_dx(j, os.environ.get('THIN', '1') == '1')
            r0 = _row_tile(j)
            rd = pl.multiple_of(jnp.where(j < 5, r0, D), 64)
            tin = dwq_s[pl.ds(r0, 128), :]
            if os.environ.get('GATE2', '0') == '1':
                head = jnp.concatenate([tin[0:16, 0:128] + link * 0.0, tin[0:16, 128:]], axis=1)
                tin = jnp.concatenate([head, tin[16:]], axis=0)
            tb = tin.T
            for gi, grp in enumerate(GROUPS):
                if grp is None:
                    continue
                tt, d = grp
                tmp_s[pl.ds(tt * D + d, 32, stride=DH), :] = tb[gi * 32:(gi + 1) * 32, :]
            dwqkv_s[pl.ds(rd, 128), :] = tmp_s[pl.ds(0, 3 * D), :].astype(bf16).T
            out_copy(outT_s, outT_hbm, j, 0).start()

            out_copy(dxT_s, dxT_hbm, j, 1).start()

            @pl.when(j == 4)
            def _():
                dwqkv_copy.start()
            return carry

        with jax.named_scope('fin_loop'):
            jax.lax.fori_loop(0, NB, fin_body, 0)
        dwo_copy.wait()
        db1_copy.wait()
        db2_copy.wait()
        dwqkv_copy.wait()
        for j in range(NB):
            out_copy(outT_s, outT_hbm, j, 0).wait()
            out_copy(dxT_s, dxT_hbm, j, 1).wait()
        for c in range(NF):
            dw_copy(dw1_s, dw1_hbm, c, 0).wait()
            dw_copy(dw2T_s, dw2T_hbm, c, 1).wait()

    with jax.named_scope('tail'):
        _tail()


def _full(shape):
    return pl.BlockSpec(shape, lambda c: (0,) * len(shape))


@jax.jit
def pallas_parallel_sum__sliding_local_dilated__mixer_channel_mlp__prompt_kernel(A_x, A_wqkv, A_wo, B_x, B_w1, B_b1, B_w2, B_b2, grad_out):
    xT = A_x.reshape(S, D).T
    gT = grad_out.reshape(S, D).T
    w2T = B_w2.T
    anyspec = pl.BlockSpec(memory_space=pl.ANY)
    vmemspec = pl.BlockSpec(memory_space=pltpu.VMEM)
    outs = pl.pallas_call(
        kernel,
        in_specs=[anyspec] * 1 + [anyspec] * 6 + [anyspec],
        out_specs=[anyspec] * 1 + [anyspec] * 6 + [anyspec],
        out_shape=[jax.ShapeDtypeStruct((D, S), bf16), jax.ShapeDtypeStruct((D, S), bf16),
                   jax.ShapeDtypeStruct((D, 3 * D), bf16), jax.ShapeDtypeStruct((D, D), bf16),
                   jax.ShapeDtypeStruct((D, F), bf16), jax.ShapeDtypeStruct((F,), bf16),
                   jax.ShapeDtypeStruct((D, F), bf16), jax.ShapeDtypeStruct((D,), bf16)],
        scratch_shapes=[
            pltpu.VMEM((F,), bf16),
            pltpu.VMEM((D,), bf16),
            pltpu.VMEM((F,), bf16),
            pltpu.VMEM((D,), bf16),
            pltpu.VMEM((D, S), bf16),
            pltpu.VMEM((D, S), bf16),
            pltpu.VMEM((D, 3 * D), bf16),
            pltpu.VMEM((D, D), bf16),
            pltpu.VMEM((D, F), bf16),
            pltpu.VMEM((D, F), bf16),
            pltpu.VMEM((D, F), bf16),
            pltpu.VMEM((D, F), bf16),
            pltpu.VMEM((D + 128, 3 * D), bf16),
            pltpu.VMEM((D, D), bf16),
            pltpu.VMEM((D, DP), bf16),
            pltpu.VMEM((D, S), bf16),
            pltpu.VMEM((D, S), bf16),
            pltpu.VMEM((S, D), bf16),
            pltpu.VMEM((S, D), bf16),
            pltpu.VMEM((S, D), bf16),
            pltpu.VMEM((8, S), f32),
            pltpu.VMEM((D, QP), bf16),
            pltpu.VMEM((D, DP), bf16),
            pltpu.VMEM((QP, 128), f32),
            pltpu.VMEM((8, DP), f32),
            pltpu.VMEM((NQ + 5, S + PAD, 128), f32),
            pltpu.VMEM((S + RS, QP), bf16),
            pltpu.VMEM((S, DP), bf16),
            pltpu.VMEM((D, S), f32),
            pltpu.VMEM((D, S), f32),
            pltpu.VMEM((D, QP), f32),
            pltpu.VMEM((DP, DP), f32),
            pltpu.VMEM((D, TB), f32),
            pltpu.VMEM((5, RS + PAD, 128), f32),
            pltpu.VMEM((5, RS + PAD, 128), f32),
            pltpu.VMEM((6, 2 * RS + PAD, 128), f32),
            pltpu.VMEM((5, 2 * RS + PAD, 128), f32),
            pltpu.VMEM((W, 2 * RS + PAD, 128), f32),
            pltpu.VMEM((W, 2 * RS + PAD, 128), f32),
            pltpu.SemaphoreType.DMA((4, NB)),
            pltpu.SemaphoreType.DMA((3, NB)),
            pltpu.SemaphoreType.DMA((2, NF)),
        ],
        compiler_params=pltpu.CompilerParams(vmem_limit_bytes=124 * 1024 * 1024),
    )(xT, gT, A_wqkv, A_wo, B_w1, B_b1, w2T, B_b2)
    outT, dxT, dwqkv, dwo, dw1, db1, dw2T, db2 = outs
    return (outT.T.reshape(1, S, D), dxT.T.reshape(1, S, D), dwqkv, dwo, dw1, db1, dw2T.T, db2)
```

```python
import functools
import os
import jax
import jax.numpy as jnp
import jax.experimental.pallas as pl
import jax.experimental.pallas.tpu as pltpu

S, D, F = 2048, 576, 4608
H, DH, W, DIL = 32, 18, 8, 2
DP = 640
NQ = 14
QP = NQ * 128
PAD = 16
EPS = 1e-5
SCALE = DH ** -0.5
C0 = 0.7978845608028654
C1 = 0.044715
NEG = -1e9

TF = int(os.environ.get('TF', 384))
NF = F // TF
TB = 256
NB = S // TB
RA = 8
RS = int(os.environ.get('RS', 192))
NSL = -(-S // RS)
FP = NSL * RS - S
assert NSL + 1 <= NF
NOSER = int(os.environ.get('NOSER', 4))

f32 = jnp.float32
bf16 = jnp.bfloat16


def NN(a, b):
    return jax.lax.dot_general(a, b, (((1,), (0,)), ((), ())), preferred_element_type=f32)


def NT(a, b):
    return jax.lax.dot_general(a, b, (((1,), (1,)), ((), ())), preferred_element_type=f32)


GROUPS = ([(0, d) for d in range(16)] + [(1, d) for d in range(16)] + [(2, d) for d in range(16)]
          + [(2, 16), (2, 17), (1, 16), (1, 17), None, None, (0, 16), (0, 17)])
WQ_PIECES = ((0, 128), (128, 128), (256, 128), (384, 192))


def _row_tile(j):
    return pl.multiple_of(jnp.minimum(j * 128, D - 128), 64)


def _colmean(x):
    return jnp.sum(x, axis=0, keepdims=True) * (1.0 / D)


def _head_reduce(p):
    p = p + pltpu.roll(p, 64, 1)
    return p + pltpu.roll(p, 32, 1)


def kernel(xT_hbm, gT_hbm, wqkv_hbm, wo_hbm, w1_hbm, b1_hbm, w2T_hbm, b2_hbm,
           outT_hbm, dxT_hbm, dwqkv_hbm, dwo_hbm, dw1_hbm, db1_hbm, dw2T_hbm, db2_hbm,
           b1_ref, b2_ref, db1_ref, db2_ref, bf_s,
           xT_s, gT_s, wqkv_s, wo_s, w1_s, w2T_s, dw1_s, dw2T_s, dwqkv_s, dwo_s, dwo_t,
           xnT_s, yT_s, xn_s, y_s, g_s, stats_s, wq_s, woT_s, tmp_s, tmp2_s,
           P_s, dqkv_s, o_s, oacc_s, dyacc_s, dwq_s, dwoT_s, dxn_s,
           WK, WV, WQ, WDO, WA, WDL,
           sem_in, sem_out, sem_dw):
    outT_s = xnT_s
    dxT_s = yT_s

    def blk(j):
        return pl.ds(pl.multiple_of(j * TB, TB), TB)

    def in_copy(src, dst, j, k):
        return pltpu.make_async_copy(src.at[:, blk(j)], dst.at[:, blk(j)], sem_in.at[k, j])

    def out_copy(src, dst, j, k):
        return pltpu.make_async_copy(src.at[:, blk(j)], dst.at[:, blk(j)], sem_out.at[k, j])

    def wqkv_copy(i):
        r0, n = WQ_PIECES[i]
        return pltpu.make_async_copy(wqkv_hbm.at[pl.ds(r0, n), :], wqkv_s.at[pl.ds(r0, n), :], sem_in.at[2, 1 + i])

    def chunk(c):
        return pl.ds(pl.multiple_of(c * TF, 128), TF)

    def dw_copy(src, dst, c, k):
        return pltpu.make_async_copy(src.at[:, chunk(c)], dst.at[:, chunk(c)], sem_dw.at[k, c])

    b1_copy = pltpu.make_async_copy(b1_hbm, b1_ref, sem_in.at[2, 7])
    b2_copy = pltpu.make_async_copy(b2_hbm, b2_ref, sem_in.at[3, 0])
    db1_copy = pltpu.make_async_copy(db1_ref, db1_hbm, sem_out.at[2, 2])
    db2_copy = pltpu.make_async_copy(db2_ref, db2_hbm, sem_out.at[2, 3])
    w1_copy = pltpu.make_async_copy(w1_hbm, w1_s, sem_in.at[2, 5])
    w2_copy = pltpu.make_async_copy(w2T_hbm, w2T_s, sem_in.at[2, 6])
    wo_copy = pltpu.make_async_copy(wo_hbm, wo_s, sem_in.at[2, 0])
    dwo_copy = pltpu.make_async_copy(dwo_s, dwo_hbm, sem_out.at[2, 0])
    dwqkv_copy = pltpu.make_async_copy(dwqkv_s.at[pl.ds(0, D), :], dwqkv_hbm, sem_out.at[2, 1])

    def ln_block(j):
        cols = blk(j)
        x = xT_s[:, cols].astype(f32)
        m1 = _colmean(x)
        xc = x - m1
        v1 = _colmean(xc * xc)
        r1 = jax.lax.rsqrt(v1 + EPS)
        v2 = v1 * r1 * r1
        r2 = jax.lax.rsqrt(v2 + EPS)
        stats_s[0:1, cols] = m1
        stats_s[1:2, cols] = r1
        stats_s[2:3, cols] = v2
        stats_s[3:4, cols] = r2
        xnb = (xc * r1).astype(bf16)
        yb = (xc * (r1 * r2)).astype(bf16)
        xnT_s[:, cols] = xnb
        yT_s[:, cols] = yb
        xn_s[cols, :] = xnb.T
        y_s[cols, :] = yb.T

    def _prologue():
        b2_copy.start()
        wo_copy.start()
        in_copy(gT_hbm, gT_s, 0, 1).start()
        for i in range(4):
            in_copy(gT_hbm, gT_s, i + 1, 1).start()
            wqkv_copy(i).start()
        for j in range(5, NB):
            in_copy(gT_hbm, gT_s, j, 1).start()
        for j in range(NB):
            in_copy(xT_hbm, xT_s, j, 0).start()
        w1_copy.start()
        w2_copy.start()
        b1_copy.start()
        for t in range(NQ + 5):
            P_s[t, pl.ds(0, FP + PAD), :] = jnp.zeros((FP + PAD, 128), f32)
        dwoT_s[pl.ds(D, DP - D), :] = jnp.zeros((DP - D, DP), f32)
        zw = jnp.zeros((RS + PAD, 128), f32)
        for w in range(W):
            WA[w, pl.ds(0, RS + PAD), :] = zw
            WDL[w, pl.ds(0, RS + PAD), :] = zw
        for t in (0, 1, 2, 3, 5):
            WQ[t, pl.ds(0, RS + PAD), :] = zw
        for t in range(4):
            WDO[t, pl.ds(0, RS + PAD), :] = zw
        wo_copy.wait()
        b2_copy.wait()
        b2row = b2_ref[...].astype(f32).reshape(1, D)
        for j in range(5):
            wd = 128 if j < 4 else 64
            base = (j % 2) * D
            if j == 4:
                tmp_s[pl.ds(base, D), :] = jnp.zeros((D, 128), f32)
            tmp_s[pl.ds(base, D), pl.ds(0, wd)] = wo_s[:, pl.ds(j * 128, wd)].astype(f32)
            parts = [tmp_s[pl.ds(base + d, 32, stride=DH), :] for d in range(DH)]
            brow = b2row[:, j * 128:j * 128 + wd]
            if wd < 128:
                brow = jnp.concatenate([brow, jnp.zeros((1, 128 - wd), f32)], axis=1)
            row = jax.lax.broadcasted_iota(jnp.int32, (64, 128), 0)
            parts.append(jnp.where(row == 0, jnp.broadcast_to(brow, (64, 128)), 0.0))
            wblk = jnp.concatenate(parts, axis=0).astype(bf16).T
            woT_s[pl.ds(j * 128, wd), :] = wblk[:wd]

        in_copy(gT_hbm, gT_s, 0, 1).wait()
        g_s[blk(0), :] = gT_s[:, blk(0)].T

        def do_block(j):
            jn = jnp.minimum(j + 1, NB - 1)
            do = NN(g_s[blk(j), :], woT_s[...])
            g_s[blk(jn), :] = gT_s[:, blk(jn)].T
            prow = pl.ds(pl.multiple_of(j * TB + FP + PAD, PAD), TB)
            for t in range(5):
                P_s[NQ + t, prow, :] = do[:, t * 128:(t + 1) * 128]

        def p2a_body(j, carry):
            in_copy(gT_hbm, gT_s, j + 1, 1).wait()
            for i in range(4):
                @pl.when(j == i)
                def _():
                    wqkv_copy(i).wait()
            do_block(j)
            r0 = _row_tile(j)
            tmp_s[pl.ds(0, 3 * D), :] = wqkv_s[pl.ds(r0, 128), :].T.astype(f32)
            parts = []
            for grp in GROUPS:
                if grp is None:
                    parts.append(jnp.zeros((32, 128), f32))
                else:
                    t, d = grp
                    parts.append(tmp_s[pl.ds(t * D + d, 32, stride=DH), :])
            wq_s[pl.ds(r0, 128), :] = jnp.concatenate(parts, axis=0).astype(bf16).T
            return carry

        def p2b_body(j, carry):
            @pl.when(j < NB - 1)
            def _():
                in_copy(gT_hbm, gT_s, jnp.minimum(j + 1, NB - 1), 1).wait()
            in_copy(xT_hbm, xT_s, j - 5, 0).wait()
            do_block(j)
            ln_block(j - 5)
            return carry

        with jax.named_scope('p2_loop'):
            jax.lax.fori_loop(0, 5, p2a_body, 0)
            jax.lax.fori_loop(5, NB, p2b_body, 0)

        def p3_body(j, carry):
            jn = jnp.minimum(j + 3, NB - 1)

            @pl.when(j + 3 < NB)
            def _():
                in_copy(xT_hbm, xT_s, jn, 0).wait()
            qkv = NN(xn_s[blk(j), :], wq_s[...])
            prow = pl.ds(pl.multiple_of(j * TB + FP + PAD, PAD), TB)
            for t in range(NQ):
                P_s[t, prow, :] = qkv[:, t * 128:(t + 1) * 128]
            ln_block(jn)
            return carry

        with jax.named_scope('p3_loop'):
            jax.lax.fori_loop(0, NB, p3_body, 0)

    with jax.named_scope('prologue'):
        _prologue()
        w1_copy.wait()
        w2_copy.wait()
        b1_copy.wait()
        bf_s[0:1, :] = b1_ref[...].astype(f32).reshape(1, F)

    lane = jax.lax.broadcasted_iota(jnp.int32, (RA, 128), 1)

    def chain(ms, load, prev):
        acc = None
        for w in range(W):
            v = ms[w] * load(w)
            if acc is None:
                acc = v if prev is None else v + prev * 0.0
            else:
                acc = acc + v
        return acc

    def attn_a2(rs, lr, ser):
        rows = pl.ds(rs + lr, RA)
        lrows = pl.ds(lr, RA)
        kr = lambda w: pl.ds(lr + PAD - DIL * w, RA)
        q = [WQ[t, lrows, :] for t in range(5)]
        do = [WDO[t, lrows, :] for t in range(5)]
        lg, da = [], []
        for w in range(W):
            p = q[0] * WK[0, kr(w), :]
            pd = do[0] * WV[0, kr(w), :]
            for t in range(1, 5):
                p = p + q[t] * WK[t, kr(w), :]
                pd = pd + do[t] * WV[t, kr(w), :]
            lg.append(_head_reduce(p))
            da.append(_head_reduce(pd))
        m = functools.reduce(jnp.maximum, lg)
        e = [jnp.exp(l - m) for l in lg]
        inv = 1.0 / functools.reduce(jnp.add, e)
        a = [x * inv for x in e]
        cc = functools.reduce(jnp.add, [a[w] * da[w] for w in range(W)])
        dl = [a[w] * (da[w] - cc) for w in range(W)]
        for w in range(W):
            WA[w, lrows, :] = a[w]
            WDL[w, lrows, :] = dl[w]
        prev = None
        for t in range(4):
            o = chain(a, lambda w: WV[t, kr(w), :], prev)
            o_s[rows, t * 128:(t + 1) * 128] = o.astype(bf16)
            dq = chain(dl, lambda w: WK[t, kr(w), :], o if ser else None)
            dqkv_s[rows, t * 128:(t + 1) * 128] = (dq * SCALE).astype(bf16)
            prev = dq if ser else None
        mix = [jnp.where(lane < 64, a[w], dl[w]) for w in range(W)]
        acc = chain(mix, lambda w: WV[4, kr(w), :], prev)
        o_s[rows, 512:640] = jnp.where(lane < 64, acc, jnp.where(lane == 64, 1.0, 0.0)).astype(bf16)
        dqkv_s[rows, 13 * 128:14 * 128] = jnp.where(lane < 64, 0.0, acc * SCALE).astype(bf16)

    def attn_a3(rs, lr, prev):
        rows = pl.ds(rs + lr, RA)
        fr = lambda w: pl.ds(RS + lr + DIL * w, RA)
        af = [WA[w, fr(w), :] for w in range(W)]
        df = [WDL[w, fr(w), :] for w in range(W)]
        for t in range(4):
            dk = chain(df, lambda w: WQ[t, fr(w), :], prev)
            dqkv_s[rows, (4 + t) * 128:(5 + t) * 128] = dk.astype(bf16)
            dv = chain(af, lambda w: WDO[t, fr(w), :], dk)
            dqkv_s[rows, (8 + t) * 128:(9 + t) * 128] = dv.astype(bf16)
            prev = dv
        mix = [jnp.where(lane < 64, af[w], df[w]) for w in range(W)]
        acc = chain(mix, lambda w: WQ[5, fr(w), :], prev)
        dqkv_s[rows, 12 * 128:13 * 128] = acc.astype(bf16)
        return acc

    def attn_slice(c):
        rs0 = pl.multiple_of(jnp.maximum(NSL - 1 - c, 0) * RS, 64)
        rs1 = pl.multiple_of(jnp.where((c >= 1) & (c <= NSL), NSL - c, NSL) * RS, 64)
        hi = pl.ds(RS, RS + PAD)
        lo = pl.ds(0, RS + PAD)
        cur = pl.ds(0, RS)
        for w in range(W):
            WA[w, hi, :] = WA[w, lo, :]
            WDL[w, hi, :] = WDL[w, lo, :]
        for t in (0, 1, 2, 3, 5):
            WQ[t, hi, :] = WQ[t, lo, :]
        for t in range(4):
            WDO[t, hi, :] = WDO[t, lo, :]
        src = pl.ds(rs0 + PAD, RS)
        srch = pl.ds(rs0, RS + PAD)
        for t in range(4):
            WQ[t, cur, :] = P_s[t, src, :] * SCALE
            WDO[t, cur, :] = P_s[NQ + t, src, :]
            WK[t] = P_s[4 + t, srch, :]
            WV[t] = P_s[8 + t, srch, :]
        ln = jax.lax.broadcasted_iota(jnp.int32, (RS, 128), 1)
        q4 = P_s[13, src, :] * SCALE
        do4 = jnp.where(ln < 64, P_s[NQ + 4, src, :], 0.0)
        WQ[4, cur, :] = jnp.where(ln < 32, 1.0, q4)
        WQ[5, cur, :] = do4 + q4
        WDO[4, cur, :] = do4
        lnh = jax.lax.broadcasted_iota(jnp.int32, (RS + PAD, 128), 1)
        rowh = jax.lax.broadcasted_iota(jnp.int32, (RS + PAD, 128), 0) + rs0
        t12 = P_s[12, srch, :]
        WV[4] = t12
        WK[4] = jnp.where(lnh < 64, jnp.where((lnh < 32) & (rowh < FP + PAD), NEG, 0.0), t12)
        p = None
        for b in reversed(range(RS // RA)):
            p = attn_a3(rs1, b * RA, p)
        for b in reversed(range(RS // RA)):
            attn_a2(rs0, b * RA, b >= NOSER)

    def mlp_body(c, carry):
        attn_slice(c)
        ck = chunk(c)
        w1c = w1_s[:, ck]
        w2c = w2T_s[:, ck]
        b1c = bf_s[0:1, ck]
        hpre = NN(y_s[...], w1c) + b1c
        dh = NN(g_s[...], w2c)
        x2 = hpre * hpre
        t = jnp.tanh(hpre * (C0 + (C0 * C1) * x2))
        hx = 0.5 * hpre
        opt = 1.0 + t
        hb = (hx * opt).astype(bf16)
        gp = 0.5 * opt + hx * (1.0 - t * t) * (C0 + (3 * C0 * C1) * x2)
        dhp = dh * gp
        bf_s[1:2, ck] = jnp.sum(dhp, axis=0, keepdims=True)
        dhb = dhp.astype(bf16)
        oacc_s[...] = jnp.where(c > 0, oacc_s[...], 0.0) + NT(w2c, hb)
        dyacc_s[...] = jnp.where(c > 0, dyacc_s[...], 0.0) + NT(w1c, dhb)
        dw2T_s[:, ck] = NN(gT_s[...], hb).astype(bf16)
        dw1_s[:, ck] = NN(yT_s[...], dhb).astype(bf16)
        dw_copy(dw1_s, dw1_hbm, c, 0).start()
        dw_copy(dw2T_s, dw2T_hbm, c, 1).start()
        return carry

    with jax.named_scope('mlp'):
        jax.lax.fori_loop(0, NF, mlp_body, 0)

    def _tail():
        db1_ref[...] = bf_s[1:2, :].reshape(F).astype(bf16)
        db1_copy.start()
        def dwo_body(n, carry):
            cols = pl.ds(pl.multiple_of(n * 128, 128), 128)
            dwoT_s[pl.ds(0, D), cols] = NN(gT_s[...], o_s[pl.ds(FP, S), cols])
            return carry

        with jax.named_scope('dwo_loop'):
            jax.lax.fori_loop(0, 5, dwo_body, 0)

        def dwq_body(n, carry):
            cols = pl.ds(pl.multiple_of(n * 256, 256), 256)
            dwq_s[:, cols] = NN(xnT_s[...], dqkv_s[pl.ds(FP, S), cols])
            jt = jnp.minimum(n, 4)
            r0 = pl.multiple_of(jt * 128, 128)
            tb = dwoT_s[pl.ds(r0, 128), :].T
            for d in range(DH):
                tmp_s[pl.ds(d, 32, stride=DH), :] = tb[d * 32:(d + 1) * 32, :]
            dwo_t[:, pl.ds(r0, 128)] = tmp_s[pl.ds(0, D), :].astype(bf16)
            tmp2_s[:, pl.ds(r0, 128)] = tb[D:D + 8, :]
            return carry

        with jax.named_scope('dwq_loop'):
            jax.lax.fori_loop(0, NQ // 2, dwq_body, 0)
        db2_ref[...] = tmp2_s[0:1, 0:D].reshape(D).astype(bf16)
        dwo_s[...] = dwo_t[:, 0:D]
        dwo_copy.start()
        db2_copy.start()

        def fin_dx(j, thin):
            RC = 16
            bc = lambda v: jnp.broadcast_to(v, (RC, 128))
            red = lambda v: jnp.sum(v, axis=0, keepdims=True) * (1.0 / D)
            link = None
            for h in range(TB // 128):
                if os.environ.get('HL', '0') == '0':
                    link = None
                cols = pl.ds(pl.multiple_of(j * TB + h * 128, 128), 128)
                lc = pl.ds(h * 128, 128)
                m1 = stats_s[0:1, cols]
                r1 = stats_s[1:2, cols]
                v2 = stats_s[2:3, cols]
                r2 = stats_s[3:4, cols]
                m1b, r1b, r2b = bc(m1), bc(r1), bc(r2)
                su = sux = sb = None
                for k in range(D // RC):
                    rr = pl.ds(k * RC, RC)
                    mk = m1b if (link is None or not thin) else m1b + link * 0.0
                    xn = (xT_s[rr, cols].astype(f32) - mk) * r1b
                    dy = dyacc_s[rr, cols]
                    u = dxn_s[rr, lc] + r2b * dy
                    su = u if su is None else su + u
                    sux = u * xn if sux is None else sux + u * xn
                    sb = dy * xn if sb is None else sb + dy * xn
                    link = sux
                k0 = bc(red(su))
                k1 = bc(red(sux) + (r2 * r2 * r2) * (1.0 - v2) * red(sb))
                for k in range(D // RC):
                    rr = pl.ds(k * RC, RC)
                    mk = m1b if not thin else m1b + link * 0.0
                    xn = (xT_s[rr, cols].astype(f32) - mk) * r1b
                    u = dxn_s[rr, lc] + r2b * dyacc_s[rr, cols]
                    dx = r1b * (u - k0 - xn * k1)
                    dxT_s[rr, cols] = (gT_s[rr, cols].astype(f32) + dx).astype(bf16)
                    link = dx
            return link

        def fin_body(j, carry):
            cols = blk(j)
            arows = pl.ds(pl.multiple_of(j * TB + FP, 64), TB)
            dxn_s[...] = NT(wq_s[...], dqkv_s[arows, :])
            outT_s[:, cols] = (oacc_s[:, cols] + xT_s[:, cols].astype(f32) + NT(woT_s[...], o_s[arows, :])).astype(bf16)
            link = fin_dx(j, os.environ.get('THIN', '1') == '1')
            r0 = _row_tile(j)
            rd = pl.multiple_of(jnp.where(j < 5, r0, D), 64)
            tin = dwq_s[pl.ds(r0, 128), :]
            if os.environ.get('GATE2', '0') == '1':
                head = jnp.concatenate([tin[0:16, 0:128] + link * 0.0, tin[0:16, 128:]], axis=1)
                tin = jnp.concatenate([head, tin[16:]], axis=0)
            tb = tin.T
            for gi, grp in enumerate(GROUPS):
                if grp is None:
                    continue
                tt, d = grp
                tmp_s[pl.ds(tt * D + d, 32, stride=DH), :] = tb[gi * 32:(gi + 1) * 32, :]
            dwqkv_s[pl.ds(rd, 128), :] = tmp_s[pl.ds(0, 3 * D), :].astype(bf16).T
            out_copy(outT_s, outT_hbm, j, 0).start()

            out_copy(dxT_s, dxT_hbm, j, 1).start()

            @pl.when(j == 4)
            def _():
                dwqkv_copy.start()
            return carry

        with jax.named_scope('fin_loop'):
            jax.lax.fori_loop(0, NB, fin_body, 0)
        dwo_copy.wait()
        db1_copy.wait()
        db2_copy.wait()
        dwqkv_copy.wait()
        for j in range(NB):
            out_copy(outT_s, outT_hbm, j, 0).wait()
            out_copy(dxT_s, dxT_hbm, j, 1).wait()
        for c in range(NF):
            dw_copy(dw1_s, dw1_hbm, c, 0).wait()
            dw_copy(dw2T_s, dw2T_hbm, c, 1).wait()

    with jax.named_scope('tail'):
        _tail()


def _full(shape):
    return pl.BlockSpec(shape, lambda c: (0,) * len(shape))


@jax.jit
def pallas_parallel_sum__sliding_local_dilated__mixer_channel_mlp__prompt_kernel(A_x, A_wqkv, A_wo, B_x, B_w1, B_b1, B_w2, B_b2, grad_out):
    xT = A_x.reshape(S, D).T
    gT = grad_out.reshape(S, D).T
    w2T = B_w2.T
    anyspec = pl.BlockSpec(memory_space=pl.ANY)
    vmemspec = pl.BlockSpec(memory_space=pltpu.VMEM)
    outs = pl.pallas_call(
        kernel,
        in_specs=[anyspec] * 1 + [anyspec] * 6 + [anyspec],
        out_specs=[anyspec] * 1 + [anyspec] * 6 + [anyspec],
        out_shape=[jax.ShapeDtypeStruct((D, S), bf16), jax.ShapeDtypeStruct((D, S), bf16),
                   jax.ShapeDtypeStruct((D, 3 * D), bf16), jax.ShapeDtypeStruct((D, D), bf16),
                   jax.ShapeDtypeStruct((D, F), bf16), jax.ShapeDtypeStruct((F,), bf16),
                   jax.ShapeDtypeStruct((D, F), bf16), jax.ShapeDtypeStruct((D,), bf16)],
        scratch_shapes=[
            pltpu.VMEM((F,), bf16),
            pltpu.VMEM((D,), bf16),
            pltpu.VMEM((F,), bf16),
            pltpu.VMEM((D,), bf16),
            pltpu.VMEM((8, F), f32),
            pltpu.VMEM((D, S), bf16),
            pltpu.VMEM((D, S), bf16),
            pltpu.VMEM((D, 3 * D), bf16),
            pltpu.VMEM((D, D), bf16),
            pltpu.VMEM((D, F), bf16),
            pltpu.VMEM((D, F), bf16),
            pltpu.VMEM((D, F), bf16),
            pltpu.VMEM((D, F), bf16),
            pltpu.VMEM((D + 128, 3 * D), bf16),
            pltpu.VMEM((D, D), bf16),
            pltpu.VMEM((D, DP), bf16),
            pltpu.VMEM((D, S), bf16),
            pltpu.VMEM((D, S), bf16),
            pltpu.VMEM((S, D), bf16),
            pltpu.VMEM((S, D), bf16),
            pltpu.VMEM((S, D), bf16),
            pltpu.VMEM((8, S), f32),
            pltpu.VMEM((D, QP), bf16),
            pltpu.VMEM((D, DP), bf16),
            pltpu.VMEM((QP, 128), f32),
            pltpu.VMEM((8, DP), f32),
            pltpu.VMEM((NQ + 5, S + FP + PAD, 128), f32),
            pltpu.VMEM((S + FP + RS, QP), bf16),
            pltpu.VMEM((S + FP, DP), bf16),
            pltpu.VMEM((D, S), f32),
            pltpu.VMEM((D, S), f32),
            pltpu.VMEM((D, QP), f32),
            pltpu.VMEM((DP, DP), f32),
            pltpu.VMEM((D, TB), f32),
            pltpu.VMEM((5, RS + PAD, 128), f32),
            pltpu.VMEM((5, RS + PAD, 128), f32),
            pltpu.VMEM((6, 2 * RS + PAD, 128), f32),
            pltpu.VMEM((5, 2 * RS + PAD, 128), f32),
            pltpu.VMEM((W, 2 * RS + PAD, 128), f32),
            pltpu.VMEM((W, 2 * RS + PAD, 128), f32),
            pltpu.SemaphoreType.DMA((4, NB)),
            pltpu.SemaphoreType.DMA((3, NB)),
            pltpu.SemaphoreType.DMA((2, NF)),
        ],
        compiler_params=pltpu.CompilerParams(vmem_limit_bytes=124 * 1024 * 1024),
    )(xT, gT, A_wqkv, A_wo, B_w1, B_b1, w2T, B_b2)
    outT, dxT, dwqkv, dwo, dw1, db1, dw2T, db2 = outs
    return (outT.T.reshape(1, S, D), dxT.T.reshape(1, S, D), dwqkv, dwo, dw1, db1, dw2T.T, db2)
```

```python
import functools
import jax
import jax.numpy as jnp
import jax.experimental.pallas as pl
import jax.experimental.pallas.tpu as pltpu

S, D, F = 2048, 576, 4608
H, DH, W, DIL = 32, 18, 8, 2
DP = 640
NQ = 14
QP = NQ * 128
PAD = 16
EPS = 1e-5
SCALE = DH ** -0.5
C0 = 0.7978845608028654
C1 = 0.044715
NEG = -1e9

TF = 384
NF = F // TF
TB = 256
NB = S // TB
RA = 8
RS = 192
NSL = -(-S // RS)
FP = NSL * RS - S
assert NSL + 1 <= NF
NOSER = 4

f32 = jnp.float32
bf16 = jnp.bfloat16


def NN(a, b):
    return jax.lax.dot_general(a, b, (((1,), (0,)), ((), ())), preferred_element_type=f32)


def NT(a, b):
    return jax.lax.dot_general(a, b, (((1,), (1,)), ((), ())), preferred_element_type=f32)


GROUPS = ([(0, d) for d in range(16)] + [(1, d) for d in range(16)] + [(2, d) for d in range(16)]
          + [(2, 16), (2, 17), (1, 16), (1, 17), None, None, (0, 16), (0, 17)])
WQ_PIECES = ((0, 128), (128, 128), (256, 128), (384, 192))


def _row_tile(j):
    return pl.multiple_of(jnp.minimum(j * 128, D - 128), 64)


def _colmean(x):
    return jnp.sum(x, axis=0, keepdims=True) * (1.0 / D)


def _head_reduce(p):
    p = p + pltpu.roll(p, 64, 1)
    return p + pltpu.roll(p, 32, 1)


def kernel(xT_hbm, gT_hbm, wqkv_hbm, wo_hbm, w1_hbm, b1_hbm, w2T_hbm, b2_hbm,
           outT_hbm, dxT_hbm, dwqkv_hbm, dwo_hbm, dw1_hbm, db1_hbm, dw2T_hbm, db2_hbm,
           b1_ref, b2_ref, db1_ref, db2_ref, bf_s,
           xT_s, gT_s, wqkv_s, wo_s, w1_s, w2T_s, dw1_s, dw2T_s, dwqkv_s, dwo_s, dwo_t,
           xnT_s, yT_s, xn_s, y_s, g_s, stats_s, wq_s, woT_s, tmp_s, tmp2_s,
           P_s, dqkv_s, o_s, oacc_s, dyacc_s, dwq_s, dwoT_s, dxn_s,
           WK, WV, WQ, WDO, WA, WDL,
           sem_in, sem_out, sem_dw):
    outT_s = xnT_s
    dxT_s = yT_s

    def blk(j):
        return pl.ds(pl.multiple_of(j * TB, TB), TB)

    def in_copy(src, dst, j, k):
        return pltpu.make_async_copy(src.at[:, blk(j)], dst.at[:, blk(j)], sem_in.at[k, j])

    def out_copy(src, dst, j, k):
        return pltpu.make_async_copy(src.at[:, blk(j)], dst.at[:, blk(j)], sem_out.at[k, j])

    def wqkv_copy(i):
        r0, n = WQ_PIECES[i]
        return pltpu.make_async_copy(wqkv_hbm.at[pl.ds(r0, n), :], wqkv_s.at[pl.ds(r0, n), :], sem_in.at[2, 1 + i])

    def chunk(c):
        return pl.ds(pl.multiple_of(c * TF, 128), TF)

    def dw_copy(src, dst, c, k):
        return pltpu.make_async_copy(src.at[:, chunk(c)], dst.at[:, chunk(c)], sem_dw.at[k, c])

    b1_copy = pltpu.make_async_copy(b1_hbm, b1_ref, sem_in.at[2, 7])
    b2_copy = pltpu.make_async_copy(b2_hbm, b2_ref, sem_in.at[3, 0])
    db1_copy = pltpu.make_async_copy(db1_ref, db1_hbm, sem_out.at[2, 2])
    db2_copy = pltpu.make_async_copy(db2_ref, db2_hbm, sem_out.at[2, 3])
    w1_copy = pltpu.make_async_copy(w1_hbm, w1_s, sem_in.at[2, 5])
    w2_copy = pltpu.make_async_copy(w2T_hbm, w2T_s, sem_in.at[2, 6])
    wo_copy = pltpu.make_async_copy(wo_hbm, wo_s, sem_in.at[2, 0])
    dwo_copy = pltpu.make_async_copy(dwo_s, dwo_hbm, sem_out.at[2, 0])
    dwqkv_copy = pltpu.make_async_copy(dwqkv_s.at[pl.ds(0, D), :], dwqkv_hbm, sem_out.at[2, 1])

    def ln_block(j):
        cols = blk(j)
        x = xT_s[:, cols].astype(f32)
        m1 = _colmean(x)
        xc = x - m1
        v1 = _colmean(xc * xc)
        r1 = jax.lax.rsqrt(v1 + EPS)
        v2 = v1 * r1 * r1
        r2 = jax.lax.rsqrt(v2 + EPS)
        stats_s[0:1, cols] = m1
        stats_s[1:2, cols] = r1
        stats_s[2:3, cols] = v2
        stats_s[3:4, cols] = r2
        xnb = (xc * r1).astype(bf16)
        yb = (xc * (r1 * r2)).astype(bf16)
        xnT_s[:, cols] = xnb
        yT_s[:, cols] = yb
        xn_s[cols, :] = xnb.T
        y_s[cols, :] = yb.T

    def _prologue():
        b2_copy.start()
        wo_copy.start()
        in_copy(gT_hbm, gT_s, 0, 1).start()
        for i in range(4):
            in_copy(gT_hbm, gT_s, i + 1, 1).start()
            wqkv_copy(i).start()
        for j in range(5, NB):
            in_copy(gT_hbm, gT_s, j, 1).start()
        for j in range(NB):
            in_copy(xT_hbm, xT_s, j, 0).start()
        w1_copy.start()
        w2_copy.start()
        b1_copy.start()
        def init_body(t, carry):
            P_s[t, pl.ds(0, FP + PAD), :] = jnp.zeros((FP + PAD, 128), f32)
            zw = jnp.zeros((RS + PAD, 128), f32)
            lo = pl.ds(0, RS + PAD)
            WA[jnp.minimum(t, W - 1), lo, :] = zw
            WDL[jnp.minimum(t, W - 1), lo, :] = zw
            return carry

        def init_body2(t, carry):
            P_s[t + W, pl.ds(0, FP + PAD), :] = jnp.zeros((FP + PAD, 128), f32)
            P_s[jnp.minimum(t + W + 6, NQ + 4), pl.ds(0, FP + PAD), :] = jnp.zeros((FP + PAD, 128), f32)
            zw = jnp.zeros((RS + PAD, 128), f32)
            lo = pl.ds(0, RS + PAD)
            WQ[t, lo, :] = zw
            WDO[jnp.minimum(t, 4), lo, :] = zw
            return carry

        jax.lax.fori_loop(0, W, init_body, 0)
        jax.lax.fori_loop(0, 6, init_body2, 0)
        dwoT_s[pl.ds(D, DP - D), :] = jnp.zeros((DP - D, DP), f32)
        wo_copy.wait()
        b2_copy.wait()
        b2row = b2_ref[...].astype(f32).reshape(1, D)
        for j in range(5):
            wd = 128 if j < 4 else 64
            base = (j % 2) * D
            if j == 4:
                tmp_s[pl.ds(base, D), :] = jnp.zeros((D, 128), f32)
            tmp_s[pl.ds(base, D), pl.ds(0, wd)] = wo_s[:, pl.ds(j * 128, wd)].astype(f32)
            parts = [tmp_s[pl.ds(base + d, 32, stride=DH), :] for d in range(DH)]
            brow = b2row[:, j * 128:j * 128 + wd]
            if wd < 128:
                brow = jnp.concatenate([brow, jnp.zeros((1, 128 - wd), f32)], axis=1)
            row = jax.lax.broadcasted_iota(jnp.int32, (64, 128), 0)
            parts.append(jnp.where(row == 0, jnp.broadcast_to(brow, (64, 128)), 0.0))
            wblk = jnp.concatenate(parts, axis=0).astype(bf16).T
            woT_s[pl.ds(j * 128, wd), :] = wblk[:wd]

        in_copy(gT_hbm, gT_s, 0, 1).wait()
        g_s[blk(0), :] = gT_s[:, blk(0)].T

        def do_block(j):
            jn = jnp.minimum(j + 1, NB - 1)
            do = NN(g_s[blk(j), :], woT_s[...])
            g_s[blk(jn), :] = gT_s[:, blk(jn)].T
            prow = pl.ds(pl.multiple_of(j * TB + FP + PAD, PAD), TB)
            for t in range(5):
                P_s[NQ + t, prow, :] = do[:, t * 128:(t + 1) * 128]

        def p2a_body(j, carry):
            in_copy(gT_hbm, gT_s, j + 1, 1).wait()
            for i in range(4):
                @pl.when(j == i)
                def _():
                    wqkv_copy(i).wait()
            do_block(j)
            r0 = _row_tile(j)
            tmp_s[pl.ds(0, 3 * D), :] = wqkv_s[pl.ds(r0, 128), :].T.astype(f32)
            parts = []
            for grp in GROUPS:
                if grp is None:
                    parts.append(jnp.zeros((32, 128), f32))
                else:
                    t, d = grp
                    parts.append(tmp_s[pl.ds(t * D + d, 32, stride=DH), :])
            wq_s[pl.ds(r0, 128), :] = jnp.concatenate(parts, axis=0).astype(bf16).T
            return carry

        def p2b_body(j, carry):
            @pl.when(j < NB - 1)
            def _():
                in_copy(gT_hbm, gT_s, jnp.minimum(j + 1, NB - 1), 1).wait()
            in_copy(xT_hbm, xT_s, j - 5, 0).wait()
            do_block(j)
            ln_block(j - 5)
            return carry

        with jax.named_scope('p2_loop'):
            jax.lax.fori_loop(0, 5, p2a_body, 0)
            jax.lax.fori_loop(5, NB, p2b_body, 0)

        def p3_body(j, carry):
            jn = jnp.minimum(j + 3, NB - 1)

            @pl.when(j + 3 < NB)
            def _():
                in_copy(xT_hbm, xT_s, jn, 0).wait()
            qkv = NN(xn_s[blk(j), :], wq_s[...])
            prow = pl.ds(pl.multiple_of(j * TB + FP + PAD, PAD), TB)
            for t in range(NQ):
                P_s[t, prow, :] = qkv[:, t * 128:(t + 1) * 128]
            ln_block(jn)
            return carry

        with jax.named_scope('p3_loop'):
            jax.lax.fori_loop(0, NB, p3_body, 0)

    with jax.named_scope('prologue'):
        _prologue()
        w1_copy.wait()
        w2_copy.wait()
        b1_copy.wait()
        bf_s[0:1, :] = b1_ref[...].astype(f32).reshape(1, F)

    lane = jax.lax.broadcasted_iota(jnp.int32, (RA, 128), 1)

    def chain(ms, load, prev):
        acc = None
        for w in range(W):
            v = ms[w] * load(w)
            if acc is None:
                acc = v if prev is None else v + prev * 0.0
            else:
                acc = acc + v
        return acc

    def attn_a2(rs, lr, ser):
        rows = pl.ds(rs + lr, RA)
        lrows = pl.ds(lr, RA)
        kr = lambda w: pl.ds(lr + PAD - DIL * w, RA)
        q = [WQ[t, lrows, :] for t in range(5)]
        do = [WDO[t, lrows, :] for t in range(5)]
        lg, da = [], []
        for w in range(W):
            p = q[0] * WK[0, kr(w), :]
            pd = do[0] * WV[0, kr(w), :]
            for t in range(1, 5):
                p = p + q[t] * WK[t, kr(w), :]
                pd = pd + do[t] * WV[t, kr(w), :]
            lg.append(_head_reduce(p))
            da.append(_head_reduce(pd))
        m = functools.reduce(jnp.maximum, lg)
        e = [jnp.exp(l - m) for l in lg]
        inv = 1.0 / functools.reduce(jnp.add, e)
        a = [x * inv for x in e]
        cc = functools.reduce(jnp.add, [a[w] * da[w] for w in range(W)])
        dl = [a[w] * (da[w] - cc) for w in range(W)]
        for w in range(W):
            WA[w, lrows, :] = a[w]
            WDL[w, lrows, :] = dl[w]
        prev = None
        for t in range(4):
            o = chain(a, lambda w: WV[t, kr(w), :], prev)
            o_s[rows, t * 128:(t + 1) * 128] = o.astype(bf16)
            dq = chain(dl, lambda w: WK[t, kr(w), :], o if ser else None)
            dqkv_s[rows, t * 128:(t + 1) * 128] = (dq * SCALE).astype(bf16)
            prev = dq if ser else None
        mix = [jnp.where(lane < 64, a[w], dl[w]) for w in range(W)]
        acc = chain(mix, lambda w: WV[4, kr(w), :], prev)
        o_s[rows, 512:640] = jnp.where(lane < 64, acc, jnp.where(lane == 64, 1.0, 0.0)).astype(bf16)
        dqkv_s[rows, 13 * 128:14 * 128] = jnp.where(lane < 64, 0.0, acc * SCALE).astype(bf16)

    def attn_a3(rs, lr, prev):
        rows = pl.ds(rs + lr, RA)
        fr = lambda w: pl.ds(RS + lr + DIL * w, RA)
        af = [WA[w, fr(w), :] for w in range(W)]
        df = [WDL[w, fr(w), :] for w in range(W)]
        for t in range(4):
            dk = chain(df, lambda w: WQ[t, fr(w), :], prev)
            dqkv_s[rows, (4 + t) * 128:(5 + t) * 128] = dk.astype(bf16)
            dv = chain(af, lambda w: WDO[t, fr(w), :], dk)
            dqkv_s[rows, (8 + t) * 128:(9 + t) * 128] = dv.astype(bf16)
            prev = dv
        mix = [jnp.where(lane < 64, af[w], df[w]) for w in range(W)]
        acc = chain(mix, lambda w: WQ[5, fr(w), :], prev)
        dqkv_s[rows, 12 * 128:13 * 128] = acc.astype(bf16)
        return acc

    def attn_slice(c):
        rs0 = pl.multiple_of(jnp.maximum(NSL - 1 - c, 0) * RS, 64)
        rs1 = pl.multiple_of(jnp.where((c >= 1) & (c <= NSL), NSL - c, NSL) * RS, 64)
        hi = pl.ds(RS, RS + PAD)
        lo = pl.ds(0, RS + PAD)
        cur = pl.ds(0, RS)
        for w in range(W):
            WA[w, hi, :] = WA[w, lo, :]
            WDL[w, hi, :] = WDL[w, lo, :]
        for t in (0, 1, 2, 3, 5):
            WQ[t, hi, :] = WQ[t, lo, :]
        for t in range(4):
            WDO[t, hi, :] = WDO[t, lo, :]
        src = pl.ds(rs0 + PAD, RS)
        srch = pl.ds(rs0, RS + PAD)
        for t in range(4):
            WQ[t, cur, :] = P_s[t, src, :] * SCALE
            WDO[t, cur, :] = P_s[NQ + t, src, :]
            WK[t] = P_s[4 + t, srch, :]
            WV[t] = P_s[8 + t, srch, :]
        ln = jax.lax.broadcasted_iota(jnp.int32, (RS, 128), 1)
        q4 = P_s[13, src, :] * SCALE
        do4 = jnp.where(ln < 64, P_s[NQ + 4, src, :], 0.0)
        WQ[4, cur, :] = jnp.where(ln < 32, 1.0, q4)
        WQ[5, cur, :] = do4 + q4
        WDO[4, cur, :] = do4
        lnh = jax.lax.broadcasted_iota(jnp.int32, (RS + PAD, 128), 1)
        rowh = jax.lax.broadcasted_iota(jnp.int32, (RS + PAD, 128), 0) + rs0
        t12 = P_s[12, srch, :]
        WV[4] = t12
        WK[4] = jnp.where(lnh < 64, jnp.where((lnh < 32) & (rowh < FP + PAD), NEG, 0.0), t12)
        p = None
        for b in reversed(range(RS // RA)):
            p = attn_a3(rs1, b * RA, p)
        for b in reversed(range(RS // RA)):
            attn_a2(rs0, b * RA, b >= NOSER)

    def mlp_body(c, carry):
        attn_slice(c)
        ck = chunk(c)
        w1c = w1_s[:, ck]
        w2c = w2T_s[:, ck]
        b1c = bf_s[0:1, ck]
        hpre = NN(y_s[...], w1c) + b1c
        dh = NN(g_s[...], w2c)
        x2 = hpre * hpre
        t = jnp.tanh(hpre * (C0 + (C0 * C1) * x2))
        hx = 0.5 * hpre
        opt = 1.0 + t
        hb = (hx * opt).astype(bf16)
        gp = 0.5 * opt + hx * (1.0 - t * t) * (C0 + (3 * C0 * C1) * x2)
        dhp = dh * gp
        bf_s[1:2, ck] = jnp.sum(dhp, axis=0, keepdims=True)
        dhb = dhp.astype(bf16)
        oacc_s[...] = jnp.where(c > 0, oacc_s[...], 0.0) + NT(w2c, hb)
        dyacc_s[...] = jnp.where(c > 0, dyacc_s[...], 0.0) + NT(w1c, dhb)
        dw2T_s[:, ck] = NN(gT_s[...], hb).astype(bf16)
        dw1_s[:, ck] = NN(yT_s[...], dhb).astype(bf16)
        dw_copy(dw1_s, dw1_hbm, c, 0).start()
        dw_copy(dw2T_s, dw2T_hbm, c, 1).start()
        return carry

    with jax.named_scope('mlp'):
        jax.lax.fori_loop(0, NF, mlp_body, 0)

    def _tail():
        db1_ref[...] = bf_s[1:2, :].reshape(F).astype(bf16)
        db1_copy.start()
        def dwo_body(n, carry):
            cols = pl.ds(pl.multiple_of(n * 128, 128), 128)
            dwoT_s[pl.ds(0, D), cols] = NN(gT_s[...], o_s[pl.ds(FP, S), cols])
            return carry

        with jax.named_scope('dwo_loop'):
            jax.lax.fori_loop(0, 5, dwo_body, 0)

        def dwq_body(n, carry):
            cols = pl.ds(pl.multiple_of(n * 256, 256), 256)
            dwq_s[:, cols] = NN(xnT_s[...], dqkv_s[pl.ds(FP, S), cols])
            jt = jnp.minimum(n, 4)
            r0 = pl.multiple_of(jt * 128, 128)
            tb = dwoT_s[pl.ds(r0, 128), :].T
            for d in range(DH):
                tmp_s[pl.ds(d, 32, stride=DH), :] = tb[d * 32:(d + 1) * 32, :]
            dwo_t[:, pl.ds(r0, 128)] = tmp_s[pl.ds(0, D), :].astype(bf16)
            tmp2_s[:, pl.ds(r0, 128)] = tb[D:D + 8, :]
            return carry

        with jax.named_scope('dwq_loop'):
            jax.lax.fori_loop(0, NQ // 2, dwq_body, 0)
        db2_ref[...] = tmp2_s[0:1, 0:D].reshape(D).astype(bf16)
        dwo_s[...] = dwo_t[:, 0:D]
        dwo_copy.start()
        db2_copy.start()

        def fin_dx(j):
            RC = 16
            bc = lambda v: jnp.broadcast_to(v, (RC, 128))
            red = lambda v: jnp.sum(v, axis=0, keepdims=True) * (1.0 / D)
            for h in range(TB // 128):
                link = None
                cols = pl.ds(pl.multiple_of(j * TB + h * 128, 128), 128)
                lc = pl.ds(h * 128, 128)
                m1 = stats_s[0:1, cols]
                r1 = stats_s[1:2, cols]
                v2 = stats_s[2:3, cols]
                r2 = stats_s[3:4, cols]
                m1b, r1b, r2b = bc(m1), bc(r1), bc(r2)
                su = sux = sb = None
                for k in range(D // RC):
                    rr = pl.ds(k * RC, RC)
                    mk = m1b if link is None else m1b + link * 0.0
                    xn = (xT_s[rr, cols].astype(f32) - mk) * r1b
                    dy = dyacc_s[rr, cols]
                    u = dxn_s[rr, lc] + r2b * dy
                    su = u if su is None else su + u
                    sux = u * xn if sux is None else sux + u * xn
                    sb = dy * xn if sb is None else sb + dy * xn
                    link = sux
                k0 = bc(red(su))
                k1 = bc(red(sux) + (r2 * r2 * r2) * (1.0 - v2) * red(sb))
                for k in range(D // RC):
                    rr = pl.ds(k * RC, RC)
                    mk = m1b + link * 0.0
                    xn = (xT_s[rr, cols].astype(f32) - mk) * r1b
                    u = dxn_s[rr, lc] + r2b * dyacc_s[rr, cols]
                    dx = r1b * (u - k0 - xn * k1)
                    dxT_s[rr, cols] = (gT_s[rr, cols].astype(f32) + dx).astype(bf16)
                    link = dx

        def fin_body(j, carry):
            cols = blk(j)
            arows = pl.ds(pl.multiple_of(j * TB + FP, 64), TB)
            dxn_s[...] = NT(wq_s[...], dqkv_s[arows, :])
            outT_s[:, cols] = (oacc_s[:, cols] + xT_s[:, cols].astype(f32) + NT(woT_s[...], o_s[arows, :])).astype(bf16)
            fin_dx(j)
            r0 = _row_tile(j)
            rd = pl.multiple_of(jnp.where(j < 5, r0, D), 64)
            tb = dwq_s[pl.ds(r0, 128), :].T
            for gi, grp in enumerate(GROUPS):
                if grp is None:
                    continue
                tt, d = grp
                tmp_s[pl.ds(tt * D + d, 32, stride=DH), :] = tb[gi * 32:(gi + 1) * 32, :]
            dwqkv_s[pl.ds(rd, 128), :] = tmp_s[pl.ds(0, 3 * D), :].astype(bf16).T
            out_copy(outT_s, outT_hbm, j, 0).start()

            out_copy(dxT_s, dxT_hbm, j, 1).start()

            @pl.when(j == 4)
            def _():
                dwqkv_copy.start()
            return carry

        with jax.named_scope('fin_loop'):
            jax.lax.fori_loop(0, NB, fin_body, 0)
        dwo_copy.wait()
        db1_copy.wait()
        db2_copy.wait()
        dwqkv_copy.wait()
        for j in range(NB):
            out_copy(outT_s, outT_hbm, j, 0).wait()
            out_copy(dxT_s, dxT_hbm, j, 1).wait()
        for c in range(NF):
            dw_copy(dw1_s, dw1_hbm, c, 0).wait()
            dw_copy(dw2T_s, dw2T_hbm, c, 1).wait()

    with jax.named_scope('tail'):
        _tail()


@jax.jit
def pallas_parallel_sum__sliding_local_dilated__mixer_channel_mlp__prompt_kernel(A_x, A_wqkv, A_wo, B_x, B_w1, B_b1, B_w2, B_b2, grad_out):
    xT = A_x.reshape(S, D).T
    gT = grad_out.reshape(S, D).T
    w2T = B_w2.T
    anyspec = pl.BlockSpec(memory_space=pl.ANY)
    outs = pl.pallas_call(
        kernel,
        in_specs=[anyspec] * 8,
        out_specs=[anyspec] * 8,
        out_shape=[jax.ShapeDtypeStruct((D, S), bf16), jax.ShapeDtypeStruct((D, S), bf16),
                   jax.ShapeDtypeStruct((D, 3 * D), bf16), jax.ShapeDtypeStruct((D, D), bf16),
                   jax.ShapeDtypeStruct((D, F), bf16), jax.ShapeDtypeStruct((F,), bf16),
                   jax.ShapeDtypeStruct((D, F), bf16), jax.ShapeDtypeStruct((D,), bf16)],
        scratch_shapes=[
            pltpu.VMEM((F,), bf16),
            pltpu.VMEM((D,), bf16),
            pltpu.VMEM((F,), bf16),
            pltpu.VMEM((D,), bf16),
            pltpu.VMEM((8, F), f32),
            pltpu.VMEM((D, S), bf16),
            pltpu.VMEM((D, S), bf16),
            pltpu.VMEM((D, 3 * D), bf16),
            pltpu.VMEM((D, D), bf16),
            pltpu.VMEM((D, F), bf16),
            pltpu.VMEM((D, F), bf16),
            pltpu.VMEM((D, F), bf16),
            pltpu.VMEM((D, F), bf16),
            pltpu.VMEM((D + 128, 3 * D), bf16),
            pltpu.VMEM((D, D), bf16),
            pltpu.VMEM((D, DP), bf16),
            pltpu.VMEM((D, S), bf16),
            pltpu.VMEM((D, S), bf16),
            pltpu.VMEM((S, D), bf16),
            pltpu.VMEM((S, D), bf16),
            pltpu.VMEM((S, D), bf16),
            pltpu.VMEM((8, S), f32),
            pltpu.VMEM((D, QP), bf16),
            pltpu.VMEM((D, DP), bf16),
            pltpu.VMEM((QP, 128), f32),
            pltpu.VMEM((8, DP), f32),
            pltpu.VMEM((NQ + 5, S + FP + PAD, 128), f32),
            pltpu.VMEM((S + FP + RS, QP), bf16),
            pltpu.VMEM((S + FP, DP), bf16),
            pltpu.VMEM((D, S), f32),
            pltpu.VMEM((D, S), f32),
            pltpu.VMEM((D, QP), f32),
            pltpu.VMEM((DP, DP), f32),
            pltpu.VMEM((D, TB), f32),
            pltpu.VMEM((5, RS + PAD, 128), f32),
            pltpu.VMEM((5, RS + PAD, 128), f32),
            pltpu.VMEM((6, 2 * RS + PAD, 128), f32),
            pltpu.VMEM((5, 2 * RS + PAD, 128), f32),
            pltpu.VMEM((W, 2 * RS + PAD, 128), f32),
            pltpu.VMEM((W, 2 * RS + PAD, 128), f32),
            pltpu.SemaphoreType.DMA((4, NB)),
            pltpu.SemaphoreType.DMA((3, NB)),
            pltpu.SemaphoreType.DMA((2, NF)),
        ],
        compiler_params=pltpu.CompilerParams(vmem_limit_bytes=124 * 1024 * 1024),
    )(xT, gT, A_wqkv, A_wo, B_w1, B_b1, w2T, B_b2)
    outT, dxT, dwqkv, dwo, dw1, db1, dw2T, db2 = outs
    return (outT.T.reshape(1, S, D), dxT.T.reshape(1, S, D), dwqkv, dwo, dw1, db1, dw2T.T, db2)
```
